```python
import os as _os
_os.environ.setdefault("JAX_PLATFORMS", "cpu")
import jax
import jax.numpy as jnp

def _softmax(x, axis=-1):
    return jax.nn.softmax(x, axis=axis)
def _gelu(x):
    return jax.nn.gelu(x, approximate=True)
def _silu(x):
    return jax.nn.silu(x)
def _sigmoid(x):
    return jax.nn.sigmoid(x)
def _layernorm(x, axis=-1, eps=1e-5):
    m = jnp.mean(x, axis=axis, keepdims=True)
    v = jnp.var(x, axis=axis, keepdims=True)
    return (x - m) / jnp.sqrt(v + eps)
def _scatter_add(tgt, idx, src, axis=0):
    return tgt.at[idx].add(src)
def _segment_sum(src, seg, n):
    return jax.ops.segment_sum(src, seg, n)
class _Rng:
    def __init__(self, key):
        self._k = key
    def _next(self):
        self._k, sub = jax.random.split(self._k)
        return sub
    def normal(self, shape):
        return jax.random.normal(self._next(), shape, dtype=jnp.bfloat16)
    def randint(self, lo, hi, shape):
        return jax.random.randint(self._next(), shape, lo, hi, dtype=jnp.int32)
    def uniform(self, shape, lo=0.0, hi=1.0):
        return jax.random.uniform(self._next(), shape, jnp.bfloat16, lo, hi)
    def permutation(self, n):
        return jax.random.permutation(self._next(), n)


kernel_name = 'concat_heads__mha_block_cached__mha_block_cached__near_ridge'

def setup_inputs():
    _rng = _Rng(jax.random.key(int.from_bytes(__import__("os").urandom(4), "little")))
    _w = (lambda a: (lambda t: t.astype(jnp.bfloat16) if jnp.issubdtype(t.dtype, jnp.floating) else t)(jnp.asarray(a)))
    def _A_setup():
        B, Sq, D = 16, 32, 1024
        H, Sk, Dh = 32, 32, 128
        return {
            "x": _w((lambda *s: _rng.normal(s) * 0.8)(B, Sq, D)),
            "k_cache": _w((lambda *s: _rng.normal(s) * 0.8)(B, H, Sk, Dh)),
            "v_cache": _w((lambda *s: _rng.normal(s) * 0.05)(B, H, Sk, Dh)),
            "wq": _w((lambda *s: _rng.normal(s) * 0.8)(D, H * Dh) * (D ** -0.5)),
            "wo": _w((lambda *s: _rng.normal(s) * 0.05)(H * Dh, D) * ((H * Dh) ** -0.5)),
        }
    _A_in = _A_setup()

    def _B_setup():
        B, Sq, D = 16, 32, 1024
        H, Sk, Dh = 32, 32, 128
        return {
            "x": _w((lambda *s: _rng.normal(s) * 0.8)(B, Sq, D)),
            "k_cache": _w((lambda *s: _rng.normal(s) * 0.8)(B, H, Sk, Dh)),
            "v_cache": _w((lambda *s: _rng.normal(s) * 0.05)(B, H, Sk, Dh)),
            "wq": _w((lambda *s: _rng.normal(s) * 0.8)(D, H * Dh) * (D ** -0.5)),
            "wo": _w((lambda *s: _rng.normal(s) * 0.05)(H * Dh, D) * ((H * Dh) ** -0.5)),
        }
    _B_in = _B_setup()

    return {
        "A_x": _A_in["x"],
        "A_k_cache": _A_in["k_cache"],
        "A_v_cache": _A_in["v_cache"],
        "A_wq": _A_in["wq"],
        "A_wo": _A_in["wo"],
        "B_x": _B_in["x"],
        "B_k_cache": _B_in["k_cache"],
        "B_v_cache": _B_in["v_cache"],
        "B_wq": _B_in["wq"],
        "B_wo": _B_in["wo"],
    }

def reference(A_x, A_k_cache, A_v_cache, A_wq, A_wo, B_x, B_k_cache, B_v_cache, B_wq, B_wo):
    def _A_ref(x, k_cache, v_cache, wq, wo):
        B, Sq, D = x.shape
        H, Dh = 32, 128
        q = (lambda x, *d: x.transpose(*d))((x @ wq).reshape(B, Sq, H, Dh), 0, 2, 1, 3)
        scores = jnp.einsum("bhqd,bhkd->bhqk", q, k_cache) * (Dh ** -0.5)
        p = _softmax(scores, axis=-1)
        o = jnp.einsum("bhqk,bhkd->bhqd", p, v_cache)
        return (lambda x, *d: x.transpose(*d))(o, 0, 2, 1, 3).reshape(B, Sq, H * Dh) @ wo

    def _B_ref(x, k_cache, v_cache, wq, wo):
        B, Sq, D = x.shape
        H, Dh = 32, 128
        q = (lambda x, *d: x.transpose(*d))((x @ wq).reshape(B, Sq, H, Dh), 0, 2, 1, 3)
        scores = jnp.einsum("bhqd,bhkd->bhqk", q, k_cache) * (Dh ** -0.5)
        p = _softmax(scores, axis=-1)
        o = jnp.einsum("bhqk,bhkd->bhqd", p, v_cache)
        return (lambda x, *d: x.transpose(*d))(o, 0, 2, 1, 3).reshape(B, Sq, H * Dh) @ wo

    a = _A_ref(A_x, A_k_cache, A_v_cache, A_wq, A_wo)
    b = _B_ref(B_x, B_k_cache, B_v_cache, B_wq, B_wo)
    return jnp.concatenate([a, b], axis=-1)
```

```python
import jax
import jax.numpy as jnp
from jax import lax
import jax.experimental.pallas as pl
import jax.experimental.pallas.tpu as pltpu

H, DH, SK = 32, 128, 32
G4 = 4
NG = 2 * H // G4
F32 = jnp.float32
BF16 = jnp.bfloat16
SCOPES = False

STARTUP = [
    ([("x",), ("wq", 0, 2)], "Q0 Q1"),
    ([("wq", 2, 4), ("wq", 4, 6)], "Q2 Q3 Q4 Q5"),
    ([("k", 0), ("wq", 6, 8), ("v", 0), ("wq", 8, 10)],
     "S0 Q6 S1 P0 Q7 S2 P1 Q8 S3 P2 Q9"),
    ([("k", 1), ("wq", 10, 12), ("v", 1), ("wo", 0)],
     "P3 S4 Q10 S5 P4 Q11 S6 P5 O0:0:3 S7 P6 O0:3:6 P7 O0:6:8"),
    ([("k", 2), ("wq", 12, 16), ("v", 2), ("wo", 1), ("k", 3)],
     "S8 Q12 S9 P8 Q13 S10 P9 Q14 S11 P10 Q15 S12 P11 O1:0:3 S13 O1:3:6 S14 S15 O1:6:8"),
    ([("v", 3), ("wo", 2), ("wo", 3)],
     "P12 P13 P14 P15 O2:0:8 O3:0:8"),
]
N0 = 16
HG = 8
LOOP_BODY = ("Q0 Q1 S0 Q2 S1 P0 Q3 S2 P1 Q4 S3 P2 Q5 S4 P3 Q6 S5 P4 Q7 S6 P5 "
             "O0:0:3 S7 P6 O0:3:6 P7 O0:6:8 O1:0:2 O1:2:4 O1:4:6 O1:6:7 O1:7:8")
NIT = (2 * H - N0) // HG
NST = len(STARTUP)
OUT_CHUNKS = [(0, 2), (2, 4), (4, 6), (6, 7), (7, 8)]


def _kernel(ax, ak, av, awq, awo, bx, bk, bv, bwq, bwo, out_hbm,
            xbuf, wqbuf, wobuf, kbuf, vbuf, acc, ostage, sem):
    M, D = ax.shape
    srcs = ((ax, ak, av, awq, awo), (bx, bk, bv, bwq, bwo))
    gpb = H // G4

    def chunk_copy(ch, s, goff=0):
        kind = ch[0]
        if kind == "x":
            br = ch[1] if len(ch) > 1 else 0
            return pltpu.make_async_copy(srcs[br][0], xbuf.at[br], s)
        if kind == "wq":
            h0, h1 = ch[1], ch[2]
            g = h0 // G4
            assert (h1 - 1) // G4 == g
            br, hb = divmod(h0, H)
            w = (h1 - h0) * DH
            return pltpu.make_async_copy(
                srcs[br][3].at[:, pl.ds(hb * DH, w)],
                wqbuf.at[g + goff, :, pl.ds((h0 % G4) * DH, w)], s)
        g = ch[1]
        br, gb = divmod(g, gpb)
        if kind == "wo":
            return pltpu.make_async_copy(
                srcs[br][4].at[pl.ds(gb * G4 * DH, G4 * DH), :],
                wobuf.at[g + goff], s)
        src = srcs[br][1] if kind == "k" else srcs[br][2]
        dst = kbuf if kind == "k" else vbuf
        return pltpu.make_async_copy(
            src.at[:, pl.ds(gb * G4, G4)], dst.at[g + goff], s)

    def iter_chunks(g0):
        chs = []
        for g in range(g0, g0 + HG // G4):
            chs += [("wq", g * G4, g * G4 + G4), ("k", g), ("v", g)]
        for g in range(g0, g0 + HG // G4):
            chs += [("wo", g)]
        return chs

    def out_copy(br, n0, n1):
        w = (n1 - n0) * 128
        return pltpu.make_async_copy(
            ostage.at[br, :, pl.ds(n0 * 128, w)],
            out_hbm.at[:, pl.ds(br * D + n0 * 128, w)],
            sem.at[NST + NIT + 1 + br])

    for st, (chs, _) in enumerate(STARTUP):
        for ch in chs:
            chunk_copy(ch, sem.at[st]).start()
    for it in range(NIT):
        g0 = (N0 + it * HG) // G4
        if g0 == gpb:
            chunk_copy(("x", 1), sem.at[NST + NIT]).start()
        for ch in iter_chunks(g0):
            chunk_copy(ch, sem.at[NST + it]).start()

    acc[1] = jnp.zeros(acc.shape[1:], F32)

    c_exp = (DH ** -0.5) * 1.4426950408889634
    r = lax.broadcasted_iota(jnp.int32, (128, 128), 0) // 32
    l = lax.broadcasted_iota(jnp.int32, (128, 128), 1) // 32
    mask = r == l

    def make_ops(br, gbase, first_o_group, last_o_group, out_pred):
        q, s, o, ocat = {}, {}, {}, {}

        def Q(h):
            g, hh = divmod(h, G4)
            w = wqbuf[gbase + g, :, hh * DH:(hh + 1) * DH]
            q[h] = jnp.dot(xbuf[br], w, preferred_element_type=F32).astype(BF16)

        def S(h):
            g, hh = divmod(h, G4)
            ps = []
            for j in range(M // 128):
                kb = kbuf[gbase + g, 4 * j:4 * j + 4, hh].reshape(128, 128)
                sc = lax.dot_general(q[h][128 * j:128 * (j + 1)], kb,
                                     (((1,), (1,)), ((), ())),
                                     preferred_element_type=F32)
                sc = jnp.where(mask, sc, -jnp.inf)
                m = jnp.max(sc, axis=-1, keepdims=True)
                e = jnp.exp2((sc - m) * c_exp)
                den = jnp.sum(e, axis=-1, keepdims=True)
                r0 = pl.reciprocal(den, approx=True)
                rr = r0 * (2.0 - den * r0)
                ps.append((e * rr).astype(BF16))
            s[h] = ps

        def P(h):
            g, hh = divmod(h, G4)
            os_ = []
            for j in range(M // 128):
                vb = vbuf[gbase + g, 4 * j:4 * j + 4, hh].reshape(128, 128)
                os_.append(jnp.dot(s[h][j], vb,
                                   preferred_element_type=F32).astype(BF16))
            o[h] = jnp.concatenate(os_, axis=0)

        def O(g, n0, n1):
            if g not in ocat:
                ocat[g] = jnp.concatenate(
                    [o[h] for h in range(g * G4, g * G4 + G4)], axis=1)
            cols = slice(n0 * 128, n1 * 128)
            y = jnp.dot(ocat[g], wobuf[gbase + g, :, cols],
                        preferred_element_type=F32)
            if g != first_o_group:
                y = acc[br, :, cols] + y
            acc[br, :, cols] = y
            if g == last_o_group:
                ostage[br, :, cols] = y.astype(BF16)
                for b in range(2):
                    @pl.when(out_pred(b))
                    def _():
                        out_copy(b, n0, n1).start()

        def run(prog):
            for tok in prog.split():
                if tok[0] == "O":
                    O(*[int(t) for t in tok[1:].split(":")])
                else:
                    {"Q": Q, "S": S, "P": P}[tok[0]](int(tok[1:]))
        return run

    def scoped(name, fn):
        if SCOPES:
            with jax.named_scope(name):
                fn()
        else:
            fn()

    run = make_ops(0, 0, 0, None, None)
    for st, (chs, prog) in enumerate(STARTUP):
        def w():
            for ch in chs:
                chunk_copy(ch, sem.at[st]).wait()
        scoped(f"wait_st{st}", w)
        run(prog)

    it_b = (H - N0) // HG

    def body(it, carry):
        br = jnp.where(it >= it_b, 1, 0)
        gbase = N0 // G4 + it * (HG // G4)

        def w():
            @pl.when(it == it_b)
            def _():
                chunk_copy(("x", 1), sem.at[NST + NIT]).wait()
            for ch in iter_chunks(0):
                chunk_copy(ch, sem.at[NST + it], goff=gbase).wait()
        scoped("wait_loop", w)
        last_it = (it_b - 1, NIT - 1)
        make_ops(br, gbase, None, HG // G4 - 1,
                 lambda b: it == last_it[b])(LOOP_BODY)
        return carry

    lax.fori_loop(0, NIT, body, 0)

    def w():
        for b in range(2):
            for (n0, n1) in OUT_CHUNKS:
                out_copy(b, n0, n1).wait()
    scoped("wait_out", w)


@jax.jit
def pallas_concat_heads__mha_block_cached__mha_block_cached__near_ridge_kernel(
    A_x, A_k_cache, A_v_cache, A_wq, A_wo, B_x, B_k_cache, B_v_cache, B_wq, B_wo):
    B, Sq, D = A_x.shape
    M = B * Sq
    out = pl.pallas_call(
        _kernel,
        in_specs=[pl.BlockSpec(memory_space=pl.ANY)] * 10,
        out_specs=pl.BlockSpec(memory_space=pl.ANY),
        out_shape=jax.ShapeDtypeStruct((M, 2 * D), BF16),
        scratch_shapes=[
            pltpu.VMEM((2, M, D), BF16),
            pltpu.VMEM((NG, D, G4 * DH), BF16),
            pltpu.VMEM((NG, G4 * DH, D), BF16),
            pltpu.VMEM((NG, B, G4, SK, DH), BF16),
            pltpu.VMEM((NG, B, G4, SK, DH), BF16),
            pltpu.VMEM((2, M, D), F32),
            pltpu.VMEM((2, M, D), BF16),
            pltpu.SemaphoreType.DMA((NST + NIT + 3,)),
        ],
        compiler_params=pltpu.CompilerParams(
            vmem_limit_bytes=100 * 1024 * 1024),
    )(A_x.reshape(M, D), A_k_cache, A_v_cache, A_wq, A_wo,
      B_x.reshape(M, D), B_k_cache, B_v_cache, B_wq, B_wo)
    return out.reshape(B, Sq, 2 * D)
```

```python
import jax
import jax.numpy as jnp
from jax import lax
import jax.experimental.pallas as pl
import jax.experimental.pallas.tpu as pltpu

H, DH, SK = 32, 128, 32
G4 = 4
NG = 2 * H // G4
F32 = jnp.float32
BF16 = jnp.bfloat16
U32 = jnp.uint32
SCOPES = False

RA = "5241736"
TE = lambda g: " ".join(f"T{g}:{n}:36" for n in range(4))
STARTUP = [
    ([("x", 0)], "X0"),
    ([("wq", 0, 2)], f"R0:{RA}"),
    ([("wq", 2, 4), ("wq", 4, 6)], f"R2:{RA} R4:{RA}"),
    ([("wq", 6, 8), ("wq", 8, 12)], f"R6:{RA} R8:{RA} R10:{RA}"),
    ([("wq", 12, 16), ("k", 0), ("v", 0), ("wq", 16, 18)],
     "R12:5 S0 R12:2417 S1 R12:36 R14:5 P0 R14:24 S2 R14:1736 P1 R16:5 S3 R16:24 P2 R16:1736"),
    ([("k", 1), ("v", 1), ("wq", 18, 20), ("wq", 20, 24), ("k", 2)],
     "R18:5 P3 S4 R18:2417 S5 R18:3 P4 R18:6 R20:5 S6 R20:241 P5 R20:7 S7 R20:36 P6 "
     "R22:5 S8 R22:241 P7 R22:7 S9 R22:36"),
    ([("wo", 0), ("wo", 1), ("v", 2), ("k", 3)],
     "T0:0:5 S10 T0:0:2 P8 T0:0:3614 S11 T0:0:7 P9 T0:1:52 S12 T0:1:36 P10 T0:1:147 "
     "S13 T0:2:5 P11 T0:2:236 S14 T0:2:147 T0:3:5 S15 T0:3:236147"),
    ([("v", 3), ("wo", 2), ("wo", 3), ("k", 4), ("v", 4), ("k", 5)],
     "P12 P13 T2:0:3 S16 T2:0:6 P14 P15 T2:1:36 S17 T2:2:36 P16 T2:3:3 S18 T2:3:6 "
     "T2:0:52 P17 T2:0:1 S19 T2:0:47 P18 T2:1:5 S20 T2:1:2147 P19 T2:2:5 S21 T2:2:214 S22 "
     "T2:2:7 T2:3:52 S23 T2:3:147"),
    ([("v", 5), ("wo", 4), ("wo", 5)],
     "P20 P21 T4:0:36 P22 P23 T4:1:36 T4:2:36 T4:3:36 "
     "T4:0:52147 T4:1:52147 T4:2:52147 T4:3:52147"),
]
N0 = 24
HG = 8
LOOP_BODY = (
    "R0:5412736 S0 R2:541 S1 P0 R2:2736 S2 P1 R4:541 S3 P2 R4:2736 S4 P3 R6:541 "
    "S5 P4 R6:2736 S6 P5 T0:0:36 T0:1:3 S7 P6 T0:1:6 T0:2:36 T0:3:3 P7 T0:3:6 "
    "T0:0:52147 T0:1:52147 T0:2:52147 T0:3:52147")
GUARD = True
Q_LIMIT = 80.0
O_LIMIT = 3.0
NIT = (2 * H - N0) // HG
NST = len(STARTUP)


def _mm(a, b):
    return jnp.dot(a, b, preferred_element_type=F32)


def _add(a, b):
    return (a.astype(F32) + b.astype(F32)).astype(BF16)


def _sub(a, b):
    return (a.astype(F32) - b.astype(F32)).astype(BF16)


def _rhs(i, b11, b12, b21, b22):
    return {1: lambda: _add(b11(), b22()), 2: b11, 3: lambda: _sub(b12(), b22()),
            4: lambda: _sub(b21(), b11()), 5: b22, 6: lambda: _add(b11(), b12()),
            7: lambda: _add(b21(), b22())}[i]()


def _lhs(i, a11, a12, a21, a22):
    return {1: lambda: a11() + a22(), 2: lambda: a21() + a22(), 3: a11, 4: a22,
            5: lambda: a11() + a12(), 6: lambda: a21() - a11(),
            7: lambda: a12() - a22()}[i]().astype(BF16)


def _kernel(ax, ak, av, awq, awo, bx, bk, bv, bwq, bwo, out_hbm,
            xbuf, wqbuf, wobuf, kbuf, vbuf, acc, ostage, xsum, zref, sem):
    M, D = ax.shape
    hm, hk = M // 2, D // 2
    srcs = ((ax, ak, av, awq, awo), (bx, bk, bv, bwq, bwo))
    gpb = H // G4

    def chunk_copy(ch, s, goff=0):
        kind = ch[0]
        if kind == "x":
            br = ch[1] if len(ch) > 1 else 0
            return pltpu.make_async_copy(srcs[br][0], xbuf.at[br], s)
        if kind == "wq":
            h0, h1 = ch[1], ch[2]
            g = h0 // G4
            assert (h1 - 1) // G4 == g
            br, hb = divmod(h0, H)
            w = (h1 - h0) * DH
            return pltpu.make_async_copy(
                srcs[br][3].at[:, pl.ds(hb * DH, w)],
                wqbuf.at[g + goff, :, pl.ds((h0 % G4) * DH, w)], s)
        g = ch[1]
        br, gb = divmod(g, gpb)
        if kind == "wo":
            return pltpu.make_async_copy(
                srcs[br][4].at[pl.ds(gb * G4 * DH, G4 * DH), :],
                wobuf.at[g + goff], s)
        src = srcs[br][1] if kind == "k" else srcs[br][2]
        dst = kbuf if kind == "k" else vbuf
        return pltpu.make_async_copy(
            src.at[:, pl.ds(gb * G4, G4)], dst.at[g + goff], s)

    def iter_chunks(g0):
        chs = []
        for g in range(g0, g0 + HG // G4):
            chs += [("wq", g * G4, g * G4 + G4), ("k", g), ("v", g)]
        for g in range(g0, g0 + HG // G4):
            chs += [("wo", g)]
        return chs

    def out_copy(br, n):
        return pltpu.make_async_copy(
            ostage.at[br, :, pl.ds(n * 128, 128)],
            out_hbm.at[:, pl.ds(br * D + n * 128, 128)],
            sem.at[NST + NIT + br])

    for st, (chs, _) in enumerate(STARTUP):
        for ch in chs:
            chunk_copy(ch, sem.at[st]).start()
    for it in range(NIT):
        g0 = (N0 + it * HG) // G4
        if g0 == gpb:
            chunk_copy(("x", 1), sem.at[NST + NIT + 2]).start()
        for ch in iter_chunks(g0):
            chunk_copy(ch, sem.at[NST + it]).start()

    acc[1] = jnp.zeros(acc.shape[1:], F32)
    for i in range(8):
        zref[i] = 0

    c_exp = (DH ** -0.5) * 1.4426950408889634
    r = lax.broadcasted_iota(jnp.int32, (128, 128), 0) // 32
    l = lax.broadcasted_iota(jnp.int32, (128, 128), 1) // 32
    mask = r == l

    def softmax_tile(qb, kb, hook=None):
        sc = lax.dot_general(qb, kb, (((1,), (1,)), ((), ())),
                             preferred_element_type=F32)
        sc = jnp.where(mask, sc, -jnp.inf)
        m = jnp.max(sc, axis=-1, keepdims=True)
        e = jnp.exp2((sc - m) * c_exp)
        if hook is not None:
            e = hook(e)
        den = jnp.sum(e, axis=-1, keepdims=True)
        r0 = pl.reciprocal(den, approx=True)
        rr = r0 * (2.0 - den * r0)
        return (e * rr).astype(BF16)

    def X(b):
        rb = 32

        def xbody(c, carry):
            r0 = pl.multiple_of(c * rb, rb)
            blk = lambda ro, c0: xbuf[b, pl.ds(ro + r0, rb), c0:c0 + hk].astype(F32)
            vals = (blk(0, 0), blk(0, hk), blk(hm, 0), blk(hm, hk))
            blocks = [(lambda v=v: v) for v in vals]
            w0 = pl.multiple_of(c * (rb // 2), rb // 2)
            for i in range(1, 8):
                xsum[b, i - 1, pl.ds(w0, rb // 2), :] = pltpu.bitcast(
                    _lhs(i, *blocks), U32)
            return carry

        lax.fori_loop(0, hm // rb, xbody, 0)

    def make_ops(br, gbase, first_o_group, out_pred, zs, st):
        q, s, of, ocat, prods, olhs = {}, {}, {}, {}, {}, {}

        def track(name, v):
            t = jnp.max(jnp.abs(v).reshape(v.shape[0] // 8, 8, 128), axis=0)
            st[name] = jnp.maximum(st[name], t)

        def tie(name, y):
            head = jnp.where(zs[0] != 0, st[name], y[0:8])
            return jnp.concatenate([head, y[8:]], axis=0)

        def Q(h):
            g, hh = divmod(h, G4)
            w = wqbuf[gbase + g, :, hh * DH:(hh + 1) * DH]
            qf = _mm(xbuf[br], w).astype(BF16)
            q[h, 0], q[h, 1] = qf[:hm], qf[hm:]

        def combine(m, done, emit):
            for blk, need, f in (
                    ((0, 0), (1, 4, 5, 7), lambda: m[1] + m[4] - m[5] + m[7]),
                    ((0, 1), (3, 5), lambda: m[3] + m[5]),
                    ((1, 0), (2, 4), lambda: m[2] + m[4]),
                    ((1, 1), (1, 2, 3, 6), lambda: m[1] - m[2] + m[3] + m[6])):
                if blk not in done and all(i in m for i in need):
                    done.add(blk)
                    emit(blk, f())

        def R(h, which):
            g, hh = divmod(h, G4)
            blk = lambda z, r0, c: (
                lambda: wqbuf[gbase + g + z, r0:r0 + hk, c * DH:(c + 1) * DH])
            blocks = lambda z: (blk(z, 0, hh), blk(z, 0, hh + 1), blk(z, hk, hh), blk(z, hk, hh + 1))
            m, done = prods.setdefault(("R", h), ({}, set()))

            def emit(blk_, y):
                if GUARD and blk_[0] == blk_[1]:
                    y = tie("q", y)
                q[h + blk_[1], blk_[0]] = y.astype(BF16)

            for i in map(int, str(which)):
                a = pltpu.bitcast(xsum[br, i - 1], BF16)
                m[i] = _mm(a, _rhs(i, *blocks(zs[i])))
                if GUARD and i in (1, 6, 7):
                    track("q", m[i])
                combine(m, done, emit)

        def S(h):
            g, hh = divmod(h, G4)
            ps = []
            for j in range(M // 128):
                kb = kbuf[gbase + g, 4 * j:4 * j + 4, hh].reshape(128, 128)
                qb = q[h, j // 2][128 * (j % 2):128 * (j % 2 + 1)]
                hook = None
                if GUARD:
                    track("k", kb.astype(F32))
                    if j == M // 128 - 1:
                        hook = lambda e: tie("k", e)
                ps.append(softmax_tile(qb, kb, hook))
            s[h] = ps

        def P(h):
            g, hh = divmod(h, G4)
            os_ = []
            for j in range(M // 128):
                vb = vbuf[gbase + g, 4 * j:4 * j + 4, hh].reshape(128, 128)
                os_.append(_mm(s[h][j], vb))
            of[h] = jnp.concatenate(os_, axis=0)

        def o_group(g):
            return jnp.concatenate(
                [of[h] for h in range(g * G4, g * G4 + G4)], axis=1)

        def O(g, n0, n1):
            if g not in ocat:
                ocat[g] = o_group(g).astype(BF16)
            cols = slice(n0 * 128, n1 * 128)
            y = _mm(ocat[g], wobuf[gbase + g, :, cols])
            if g != first_o_group:
                y = acc[br, :, cols] + y
            acc[br, :, cols] = y

        def T(g, n, which):
            wblk = lambda gg, nn: (
                lambda: wobuf[gbase + gg, :, nn * 128:(nn + 1) * 128])
            blocks = lambda z: (wblk(g + z, n), wblk(g + z, n + 4), wblk(g + z + 1, n), wblk(g + z + 1, n + 4))
            ablk = lambda gg, r0: (lambda: o_group(gg)[r0:r0 + hm])
            ablocks = (ablk(g, 0), ablk(g + 1, 0), ablk(g, hm), ablk(g + 1, hm))
            m, done = prods.setdefault(("T", g, n), ({}, set()))

            def emit(blk_, y):
                rows = slice(blk_[0] * hm, (blk_[0] + 1) * hm)
                nn = n + 4 * blk_[1]
                cols = slice(nn * 128, (nn + 1) * 128)
                if GUARD and blk_[0] == blk_[1]:
                    y = tie("o", y)
                if g != first_o_group:
                    y = acc[br, rows, cols] + y
                acc[br, rows, cols] = y
                if out_pred is not None:
                    if GUARD:
                        track("y", y)
                        y = tie("y", y)
                    ostage[br, rows, cols] = y.astype(BF16)
                    if (1 - blk_[0], blk_[1]) in done:
                        for b in range(2):
                            @pl.when(out_pred(b))
                            def _():
                                out_copy(b, nn).start()

            for i in map(int, str(which)):
                if (g, i) not in olhs:
                    olhs[g, i] = _lhs(i, *ablocks)
                m[i] = _mm(olhs[g, i], _rhs(i, *blocks(zs[i])))
                if GUARD and i in (1, 6, 7):
                    track("o", m[i])
                combine(m, done, emit)

        def run(prog):
            for tok in prog.split():
                fn = {"Q": Q, "S": S, "P": P, "O": O, "R": R, "T": T, "X": X}[tok[0]]
                fn(*[int(t) for t in tok[1:].split(":")])
        return run

    def scoped(name, fn):
        if SCOPES:
            with jax.named_scope(name):
                fn()
        else:
            fn()

    zs = [0] * 8
    stats = {n: jnp.zeros((8, 128), F32) for n in 'koqy'}
    run = make_ops(0, 0, 0, None, zs, stats)
    for st, (chs, prog) in enumerate(STARTUP):
        def w():
            for ch in chs:
                chunk_copy(ch, sem.at[st]).wait()
        scoped(f"wait_st{st}", w)
        if st == 1:
            zs[:] = [zref[i] for i in range(8)]
        run(prog)

    it_b = (H - N0) // HG

    def body(it, carry):
        br = jnp.where(it >= it_b, 1, 0)
        gbase = N0 // G4 + it * (HG // G4)

        @pl.when(it == it_b)
        def _():
            chunk_copy(("x", 1), sem.at[NST + NIT + 2]).wait()
            X(1)

        def w():
            for ch in iter_chunks(0):
                chunk_copy(ch, sem.at[NST + it], goff=gbase).wait()
        scoped("wait_loop", w)
        last_it = (it_b - 1, NIT - 1)
        st = dict(carry)
        make_ops(br, gbase, None, lambda b: it == last_it[b], zs, st)(LOOP_BODY)
        final = jnp.logical_or(it == last_it[0], it == last_it[1])
        st["y"] = jnp.where(final, st["y"], carry["y"])
        return st

    stats = lax.fori_loop(0, NIT, body, stats)

    if GUARD:
        ok_q = jnp.max(stats["q"]) * jnp.max(stats["k"]) <= Q_LIMIT
        ok_o = jnp.max(stats["o"]) <= O_LIMIT * jnp.max(stats["y"])
        unsafe = jnp.logical_not(jnp.logical_and(ok_q, ok_o))

    def w():
        for b in range(2):
            for n in range(D // 128):
                out_copy(b, n).wait()
    scoped("wait_out", w)

    if GUARD:
        @pl.when(unsafe)
        def _():
            def plain(t, carry):
                hh, j = t // 4, t % 4
                b, g, hl = hh // H, hh // G4, hh % G4
                rows = pl.ds(pl.multiple_of(j * 128, 128), 128)
                hcol = pl.ds(pl.multiple_of(hl * DH, DH), DH)
                qb = _mm(xbuf[b, rows, :], wqbuf[g, :, hcol]).astype(BF16)
                kb = kbuf[g, pl.ds(4 * j, 4), hl].reshape(128, 128)
                vb = vbuf[g, pl.ds(4 * j, 4), hl].reshape(128, 128)
                ob = _mm(softmax_tile(qb, kb), vb).astype(BF16)
                y = _mm(ob, wobuf[g, hcol, :])
                y = jnp.where(hh % H == 0, y, acc[b, rows, :] + y)
                acc[b, rows, :] = y
                ostage[b, rows, :] = y.astype(BF16)
                return carry

            lax.fori_loop(0, 2 * H * 4, plain, 0)
            for b in range(2):
                for n in range(D // 128):
                    out_copy(b, n).start()
            w()


@jax.jit
def pallas_concat_heads__mha_block_cached__mha_block_cached__near_ridge_kernel(
    A_x, A_k_cache, A_v_cache, A_wq, A_wo, B_x, B_k_cache, B_v_cache, B_wq, B_wo):
    B, Sq, D = A_x.shape
    M = B * Sq
    out = pl.pallas_call(
        _kernel,
        in_specs=[pl.BlockSpec(memory_space=pl.ANY)] * 10,
        out_specs=pl.BlockSpec(memory_space=pl.ANY),
        out_shape=jax.ShapeDtypeStruct((M, 2 * D), BF16),
        scratch_shapes=[
            pltpu.VMEM((2, M, D), BF16),
            pltpu.VMEM((NG, D, G4 * DH), BF16),
            pltpu.VMEM((NG, G4 * DH, D), BF16),
            pltpu.VMEM((NG, B, G4, SK, DH), BF16),
            pltpu.VMEM((NG, B, G4, SK, DH), BF16),
            pltpu.VMEM((2, M, D), F32),
            pltpu.VMEM((2, M, D), BF16),
            pltpu.VMEM((2, 7, M // 4, D // 2), U32),
            pltpu.SMEM((8,), jnp.int32),
            pltpu.SemaphoreType.DMA((NST + NIT + 3,)),
        ],
        compiler_params=pltpu.CompilerParams(
            vmem_limit_bytes=100 * 1024 * 1024),
    )(A_x.reshape(M, D), A_k_cache, A_v_cache, A_wq, A_wo,
      B_x.reshape(M, D), B_k_cache, B_v_cache, B_wq, B_wo)
    return out.reshape(B, Sq, 2 * D)
```

```python
import jax
import jax.numpy as jnp
from jax import lax
import jax.experimental.pallas as pl
import jax.experimental.pallas.tpu as pltpu

H, DH, SK = 32, 128, 32
G4 = 4
NG = 2 * H // G4
HG = 8
F32 = jnp.float32
BF16 = jnp.bfloat16
U32 = jnp.uint32
SCOPES = False

RA = "5412736"
UPURE = ("a01,c01,w0,a02,b01,w1,c02,g0,b02,w2,a12,f0,c12,g1,b12,"
         "a03,f1,c03,f2,b03,a13,g2,c13,s0,g3,b13,a23,g3,c23,s1,b23,s2,w3,s3")
STARTUP = [
    ([("wq", 0, 2), ("x", 0, 0)], "Q0:0"),
    ([("x", 0, 1)], "Q0:1"),
    ([("wq", 2, 4)], f"R2:{RA}"),
    ([("wq", 4, 8)], f"R4:{RA} R6:{RA}"),
    ([("wq", 8, 12), ("k", 0)],
     "R8:5 S0 R8:2417 S1 R8:36 R10:5 S2 R10:241 S3 R10:736"),
    ([("v", 0), ("wq", 12, 16), ("k", 1), ("v", 1)],
     "P0 S4 P1 R12:541 S5 P2 P4 R12:2736 S6 P3 P5 R14:541 S7 P6 R14:2736"),
    ([("wo", 0), ("wo", 1)], "P7 U0:" + UPURE),
    ([("wq", 16, 20), ("k", 2), ("v", 2), ("wq", 20, 24), ("k", 3)],
     "R16:5 S8 R16:241 S9 P8 R16:736 S10 P9 R18:541 S11 P10 R18:2736 S12 P11 R20:541 S13 "
     "R20:2736 S14 R22:541 S15 R22:2736"),
    ([("v", 3), ("wo", 2), ("wo", 3), ("k", 4), ("v", 4), ("k", 5)],
     (
     "P12 P13 U2:a01 S16 P14 U2:c01 D2:w0 U2:b01 S17 P15 U2:w0,a02 S18 P16 U2:c02 D2:w1 U2:b02 S19 P17 "
     "U2:w1,a12 S20 P18 U2:c12 D2:w2 U2:b12 S21 P19 U2:w2,g0,f0,a03,f1,g1,c03,f2,b03,a13,g2,c13,s0,g3,b13,"
     "a23,g3,c23,s1,b23,s2,w3,s3")),
    ([("v", 5), ("wo", 4), ("wo", 5)],
     (
     "P20 S22 P21 U4:a01,c01,b01 S23 P22 U4:w0,w1,a02,c02 P23 U4:g0,b02,w2,a12,f0,c12,g1,b12,"
     "a03,f1,c03,f2,b03,a13,g2,c13,s0,g3,b13,a23,g3,c23,s1,b23,s2,w3,s3")),
]
N0 = 24
LOOP_BODY = (
    "R0:5412736 S0 R2:54 D0:w0 R2:1 S1 P0 R2:27 D0:w1 R2:3 D0:w2 R2:6 S2 P1 R4:54 D0:w3 R4:1 "
    "S3 P2 R4:27 D0:s0 R4:3 D0:s1 R4:6 S4 P3 R6:54 D0:s2 R6:1 S5 P4 R6:273 D0:s3 R6:6 S6 P5 "
    "U0:w0,a01,c01 S7 P6 U0:w1,b01,a02,c02 P7 "
    "U0:w2,g0,b02,a12,f0,c12,g1,b12,a03,f1,c03,f2,b03,s0,a13,g2,c13,g3,b13,s1,a23,g3,c23,b23,s2,w3,s3")
YCOL = 2
HC = (-1.5, -0.5, 0.5, 1.5)
GUARD = True
Q_LIMIT = 80.0
O_LIMIT = 1.5
NIT = (2 * H - N0) // HG
NST = len(STARTUP)


def _mm(a, b):
    return jnp.dot(a, b, preferred_element_type=F32)


def _add(a, b):
    return (a.astype(F32) + b.astype(F32)).astype(BF16)


def _sub(a, b):
    return (a.astype(F32) - b.astype(F32)).astype(BF16)


def _rhs(i, b11, b12, b21, b22):
    return {1: lambda: _add(b11(), b22()), 2: b11, 3: lambda: _sub(b12(), b22()),
            4: lambda: _sub(b21(), b11()), 5: b22, 6: lambda: _add(b11(), b12()),
            7: lambda: _add(b21(), b22())}[i]()


def _lhs(i, a11, a12, a21, a22):
    return {1: lambda: _add(a11(), a22()), 2: lambda: _add(a21(), a22()), 3: a11,
            4: a22, 5: lambda: _add(a11(), a12()), 6: lambda: _sub(a21(), a11()),
            7: lambda: _sub(a12(), a22())}[i]()


def _kernel(ax, ak, av, awq, awo, bx, bk, bv, bwq, bwo, out_hbm,
            xbuf, wqbuf, wobuf, kbuf, vbuf, acc, ostage, zref, sem):
    M, D = ax.shape
    hm, hk = M // 2, D // 2
    kb_ = 2 * DH
    srcs = ((ax, ak, av, awq, awo), (bx, bk, bv, bwq, bwo))
    gpb = H // G4

    def chunk_copy(ch, s, goff=0):
        kind = ch[0]
        if kind == "x":
            br = ch[1]
            if len(ch) == 2:
                return pltpu.make_async_copy(srcs[br][0], xbuf.at[br], s)
            rows = pl.ds(ch[2] * hm, hm)
            return pltpu.make_async_copy(srcs[br][0].at[rows], xbuf.at[br, rows], s)
        if kind == "wq":
            h0, h1 = ch[1], ch[2]
            g = h0 // G4
            assert (h1 - 1) // G4 == g
            br, hb = divmod(h0, H)
            w = (h1 - h0) * DH
            return pltpu.make_async_copy(
                srcs[br][3].at[:, pl.ds(hb * DH, w)],
                wqbuf.at[g + goff, :, pl.ds((h0 % G4) * DH, w)], s)
        g = ch[1]
        br, gb = divmod(g, gpb)
        if kind == "wo":
            return pltpu.make_async_copy(
                srcs[br][4].at[pl.ds(gb * G4 * DH, G4 * DH), :],
                wobuf.at[g + goff], s)
        src = srcs[br][1] if kind == "k" else srcs[br][2]
        dst = kbuf if kind == "k" else vbuf
        return pltpu.make_async_copy(
            src.at[:, pl.ds(gb * G4, G4)], dst.at[g + goff], s)

    def iter_chunks(g0):
        chs = []
        for g in range(g0, g0 + HG // G4):
            chs += [("wq", g * G4, g * G4 + G4), ("k", g), ("v", g)]
        for g in range(g0, g0 + HG // G4):
            chs += [("wo", g)]
        return chs

    def out_copy(br, r, j):
        return pltpu.make_async_copy(
            ostage.at[br, pl.ds(r * hm, hm), pl.ds(j * kb_, kb_)],
            out_hbm.at[pl.ds(r * hm, hm), pl.ds(br * D + j * kb_, kb_)],
            sem.at[NST + NIT + br])

    for st, (chs, _) in enumerate(STARTUP):
        for ch in chs:
            chunk_copy(ch, sem.at[st]).start()
    for it in range(NIT):
        g0 = (N0 + it * HG) // G4
        if g0 == gpb:
            chunk_copy(("x", 1), sem.at[NST + NIT + 2]).start()
        for ch in iter_chunks(g0):
            chunk_copy(ch, sem.at[NST + it]).start()

    def init(c, carry):
        acc[1, pl.ds(pl.multiple_of(c * 64, 64), 64), :] = jnp.zeros((64, D), F32)
        zref[c] = 0
        return carry

    lax.fori_loop(0, 8, init, 0)
    zs = [zref[i] for i in range(8)]
    never = zs[0] != 0

    c_exp = (DH ** -0.5) * 1.4426950408889634
    r = lax.broadcasted_iota(jnp.int32, (128, 128), 0) // 32
    l = lax.broadcasted_iota(jnp.int32, (128, 128), 1) // 32
    mask = r == l

    def softmax_tile(qb, kb, hook=None):
        sc = lax.dot_general(qb, kb, (((1,), (1,)), ((), ())),
                             preferred_element_type=F32)
        sc = jnp.where(mask, sc, -jnp.inf)
        m = jnp.max(sc, axis=-1, keepdims=True)
        e = jnp.exp2((sc - m) * c_exp)
        if hook is not None:
            e = hook(e)
        den = jnp.sum(e, axis=-1, keepdims=True)
        return (e * pl.reciprocal(den, approx=True)).astype(BF16)

    def make_ops(br, gbase, first_o_group, out_pred, st):
        q, s, of, prods, xl, urhs = {}, {}, {}, {}, {}, {}
        pending = []

        def track(name, v):
            t = jnp.max(jnp.abs(v).reshape(v.shape[0] // 8, 8, v.shape[1]), axis=0)
            for c in range(v.shape[1] // 128):
                st[name] = jnp.maximum(st[name], t[:, c * 128:(c + 1) * 128])

        def tie(name, y):
            head = jnp.where(never, st[name], y[0:8, 0:128])
            if y.shape[1] > 128:
                head = jnp.concatenate([head, y[0:8, 128:]], axis=1)
            return jnp.concatenate([head, y[8:]], axis=0)

        def shadow(a):
            if not pending:
                return a
            a = pltpu.bitcast(a, U32)
            c0 = 0
            parts = []
            while pending:
                y = pending.pop()
                parts.append(jnp.where(never, y, a[:, c0:c0 + y.shape[1]]))
                c0 += y.shape[1]
            if c0 < a.shape[1]:
                parts.append(a[:, c0:])
            a = jnp.concatenate(parts, axis=1) if len(parts) > 1 else parts[0]
            return pltpu.bitcast(a, BF16)

        def Q(h, r):
            g, hh = divmod(h, G4)
            w = wqbuf[gbase + g, :, hh * DH:(hh + 2) * DH]
            y = _mm(xbuf[br, r * hm:(r + 1) * hm, :], w).astype(BF16)
            q[h, r], q[h + 1, r] = y[:, :DH], y[:, DH:]

        def R(h, which):
            g, hh = divmod(h, G4)
            m, done = prods.setdefault(("R", h), ({}, set()))
            for i in map(int, str(which)):
                z = zs[i]
                if i not in xl:
                    xb = lambda r0, c0: (
                        lambda: xbuf[br + z, r0:r0 + hm, c0:c0 + hk])
                    xl[i] = _lhs(i, xb(0, 0), xb(0, hk), xb(hm, 0), xb(hm, hk))
                wb = lambda r0, c: (
                    lambda: wqbuf[gbase + g + z, r0:r0 + hk, c * DH:(c + 1) * DH])
                rhs = _rhs(i, wb(0, hh), wb(0, hh + 1), wb(hk, hh), wb(hk, hh + 1))
                m[i] = _mm(shadow(xl[i]), rhs)
                if GUARD and i in (1, 6, 7):
                    track("q", m[i])
                for blk, need, f in (
                        ((0, 0), (1, 4, 5, 7), lambda: m[1] + m[4] - m[5] + m[7]),
                        ((0, 1), (3, 5), lambda: m[3] + m[5]),
                        ((1, 0), (2, 4), lambda: m[2] + m[4]),
                        ((1, 1), (1, 2, 3, 6), lambda: m[1] - m[2] + m[3] + m[6])):
                    if blk not in done and all(k in m for k in need):
                        done.add(blk)
                        y = f()
                        if GUARD and blk[0] == blk[1]:
                            y = tie("q", y)
                        q[h + blk[1], blk[0]] = y.astype(BF16)

        def S(h):
            g, hh = divmod(h, G4)
            ps = []
            for j in range(M // 128):
                kb = kbuf[gbase + g, 4 * j:4 * j + 4, hh].reshape(128, 128)
                qb = q[h, j // 2][128 * (j % 2):128 * (j % 2 + 1)]
                hook = None
                if GUARD:
                    track("k", kb.astype(F32))
                    if j == M // 128 - 1:
                        hook = lambda e: tie("k", e)
                ps.append(softmax_tile(qb, kb, hook))
            s[h] = ps

        def P(h):
            g, hh = divmod(h, G4)
            os_ = []
            for j in range(M // 128):
                vb = vbuf[gbase + g, 4 * j:4 * j + 4, hh].reshape(128, 128)
                os_.append(_mm(s[h][j], vb))
            of[h] = jnp.concatenate(os_, axis=0)

        def u_rhs(g, kind, idx):
            if (g, kind, *idx) in urhs:
                return urhs[(g, kind, *idx)]
            z = zs[1 + len(urhs) % 7]

            def b(i, j):
                return wobuf[gbase + g + i // 2 + z,
                             (i % 2) * kb_:(i % 2 + 1) * kb_, j * kb_:(j + 1) * kb_]

            f32 = lambda i, j: b(i, j).astype(F32)
            if kind == "s":
                i, = idx
                o_ = [k for k in range(4) if k != i]
                rhs = ((f32(i, i) - f32(o_[0], i))
                       - (f32(o_[1], i) + f32(o_[2], i))).astype(BF16)
            elif kind == "w":
                i, = idx
                rhs = ((f32(i, 0) + f32(i, 1)) + (f32(i, 2) + f32(i, 3))).astype(BF16)
            else:
                i, j = idx
                rhs = {"a": lambda: b(j, i), "c": lambda: b(i, j),
                       "b": lambda: (f32(i, j) + f32(j, i)).astype(BF16)}[kind]()
            urhs[(g, kind, *idx)] = rhs
            return rhs

        def Dp(g, nm):
            pending.append(pltpu.bitcast(
                u_rhs(g, nm[0], [int(c) for c in nm[1:]]), U32))

        def U(g, names):
            P_, lhs_, part, forced, done = prods.setdefault(
                ("U", g), ({}, {}, {}, [], set()))

            def a(r, i):
                hs = (g * G4 + 2 * i, g * G4 + 2 * i + 1)
                return jnp.concatenate(
                    [of[h][r * hm:(r + 1) * hm] for h in hs], axis=1)

            def release(v):
                if "last" not in lhs_:
                    return v
                return jnp.where(never, lhs_["last"], v)

            def pair_lhs(i, j, kind):
                dl = HC[j] - HC[i]
                if (i, j, "a") not in lhs_:
                    a1i, a1j = a(1, i), a(1, j)
                    t = (release(a(0, i)) + a(0, j)) * (1.0 / HC[i])
                    la = ((t + a1i) + a1j) * (HC[i] / dl)
                    lb = la + a1j
                    lc = lb + a1i
                    for k, v in (("a", la), ("b", lb), ("c", lc)):
                        lhs_[i, j, k] = v.astype(BF16)
                return lhs_[i, j, kind]

            def emit(r, j, y):
                rows = slice(r * hm, (r + 1) * hm)
                cols = slice(j * kb_, (j + 1) * kb_)
                if GUARD:
                    y = tie("o", y)
                if g != first_o_group and r == 1:
                    y = acc[br, rows, cols] + y
                acc[br, rows, cols] = y
                if out_pred is not None:
                    if GUARD and j == YCOL:
                        track("y", y)
                        y = tie("y", y)
                    ostage[br, rows, cols] = y.astype(BF16)
                    for b_ in range(2):
                        @pl.when(out_pred(b_))
                        def _():
                            out_copy(b_, r, j).start()

            pairs = lambda j: [(min(i, j), max(i, j)) for i in range(4) if i != j]

            def fold(kind, j):
                if (kind, j) not in part:
                    if kind == "f":
                        part[kind, j] = [None, [("w", j)] + [("E", *p) for p in pairs(j)]]
                    else:
                        y0 = (None if g == first_o_group
                              else acc[br, 0:hm, j * kb_:(j + 1) * kb_])
                        part[kind, j] = [y0, [("a" if p[0] == j else "c", *p)
                                              for p in pairs(j)] + [("s", j), ("F", j)]]
                y, todo = part[kind, j]
                order = list(P_)
                avail = [t for t in todo if t in P_]
                avail.sort(key=lambda t: (t[0] != "w", order.index(t)))
                for t in avail:
                    v = P_[t]
                    if t[0] == "E" and t[1] != j:
                        y = y - v
                        continue
                    if t[0] == "F":
                        v = v * (-HC[j])
                    n = int(HC[t[2]] - HC[t[1]]) if t[0] in "ac" else 1
                    for _ in range(n):
                        y = v if y is None else y + v
                part[kind, j] = [y, [t for t in todo if t not in P_]]

            def finish():
                for i in range(4):
                    for j in range(i + 1, 4):
                        if ("E", i, j) not in P_ and all((k, i, j) in P_ for k in "abc"):
                            P_["E", i, j] = (P_["b", i, j] - P_["c", i, j]) - P_["a", i, j]
                            lhs_["last"] = P_["E", i, j]
                for j in range(4):
                    need = [("w", j)] + [("E", *p) for p in pairs(j)]
                    if not all(t in P_ for t in need):
                        continue
                    if ("F", j) not in P_:
                        fold("f", j)
                        P_["F", j] = part["f", j][0]
                        emit(1, j, P_["F", j])
                    if j not in done and ("s", j) in P_:
                        done.add(j)
                        fold("g", j)
                        emit(0, j, part["g", j][0])

            def force(lhs):
                if not forced:
                    return lhs
                w_ = pltpu.bitcast(lhs, U32)
                while forced:
                    v = pltpu.bitcast(forced.pop(), U32).reshape(hm // 16, 2, 8, kb_)
                    for hf in range(2):
                        w_ = jnp.where(never, v[:, hf].reshape(hm // 2, kb_), w_)
                return pltpu.bitcast(w_, BF16)

            for nm in names.split(","):
                kind, idx = nm[0], [int(c) for c in nm[1:]]
                if kind in "fg":
                    fold(kind, idx[0])
                    forced.append(part[kind, idx[0]][0])
                    continue
                if kind == "s":
                    lhs = (HC[idx[0]] * release(a(1, idx[0])) + a(0, idx[0])).astype(BF16)
                elif kind == "w":
                    lhs = a(1, idx[0]).astype(BF16)
                else:
                    lhs = pair_lhs(*idx, kind)
                y = _mm(shadow(force(lhs)), u_rhs(g, kind, idx))
                P_[(kind, *idx)] = lhs_["last"] = y
                if GUARD and kind in "wb":
                    track("o", y)
                finish()

        def run(prog):
            for tok in prog.split():
                args = tok[1:].split(":")
                if tok[0] in "UD":
                    {"U": U, "D": Dp}[tok[0]](int(args[0]), args[1])
                else:
                    {"Q": Q, "S": S, "P": P, "R": R}[tok[0]](*map(int, args))
        return run

    def scoped(name, fn):
        if SCOPES:
            with jax.named_scope(name):
                fn()
        else:
            fn()

    stats = {n: jnp.zeros((8, 128), F32) for n in "koqy"}
    run = make_ops(0, 0, 0, None, stats)
    for st, (chs, prog) in enumerate(STARTUP):
        def w():
            for ch in chs:
                chunk_copy(ch, sem.at[st]).wait()
        scoped(f"wait_st{st}", w)
        run(prog)

    it_b = (H - N0) // HG

    def body(it, carry):
        br = jnp.where(it >= it_b, 1, 0)
        gbase = N0 // G4 + it * (HG // G4)

        def w():
            @pl.when(it == it_b)
            def _():
                chunk_copy(("x", 1), sem.at[NST + NIT + 2]).wait()
            for ch in iter_chunks(0):
                chunk_copy(ch, sem.at[NST + it], goff=gbase).wait()
        scoped("wait_loop", w)
        last_it = (it_b - 1, NIT - 1)
        st = dict(carry)
        make_ops(br, gbase, None, lambda b: it == last_it[b], st)(LOOP_BODY)
        final = jnp.logical_or(it == last_it[0], it == last_it[1])
        st["y"] = jnp.where(final, st["y"], carry["y"])
        return st

    stats = lax.fori_loop(0, NIT, body, stats)

    if GUARD:
        ok_q = jnp.max(stats["q"]) * jnp.max(stats["k"]) <= Q_LIMIT
        ok_o = jnp.max(stats["o"]) <= O_LIMIT * jnp.max(stats["y"])
        unsafe = jnp.logical_not(jnp.logical_and(ok_q, ok_o))

    def w():
        for b in range(2):
            for r_ in range(2):
                for j in range(4):
                    out_copy(b, r_, j).wait()
    scoped("wait_out", w)

    if GUARD:
        @pl.when(unsafe)
        def _():
            def plain(t, carry):
                hh, j = t // 4, t % 4
                b, g, hl = hh // H, hh // G4, hh % G4
                rows = pl.ds(pl.multiple_of(j * 128, 128), 128)
                hcol = pl.ds(pl.multiple_of(hl * DH, DH), DH)
                qb = _mm(xbuf[b, rows, :], wqbuf[g, :, hcol]).astype(BF16)
                kb = kbuf[g, pl.ds(4 * j, 4), hl].reshape(128, 128)
                vb = vbuf[g, pl.ds(4 * j, 4), hl].reshape(128, 128)
                ob = _mm(softmax_tile(qb, kb), vb).astype(BF16)
                y = _mm(ob, wobuf[g, hcol, :])
                y = jnp.where(hh % H == 0, y, acc[b, rows, :] + y)
                acc[b, rows, :] = y
                ostage[b, rows, :] = y.astype(BF16)
                return carry

            lax.fori_loop(0, 2 * H * 4, plain, 0)
            for b in range(2):
                for r_ in range(2):
                    for j in range(4):
                        out_copy(b, r_, j).start()
            w()


@jax.jit
def pallas_concat_heads__mha_block_cached__mha_block_cached__near_ridge_kernel(
    A_x, A_k_cache, A_v_cache, A_wq, A_wo, B_x, B_k_cache, B_v_cache, B_wq, B_wo):
    B, Sq, D = A_x.shape
    M = B * Sq
    out = pl.pallas_call(
        _kernel,
        in_specs=[pl.BlockSpec(memory_space=pl.ANY)] * 10,
        out_specs=pl.BlockSpec(memory_space=pl.ANY),
        out_shape=jax.ShapeDtypeStruct((M, 2 * D), BF16),
        scratch_shapes=[
            pltpu.VMEM((2, M, D), BF16),
            pltpu.VMEM((NG, D, G4 * DH), BF16),
            pltpu.VMEM((NG, G4 * DH, D), BF16),
            pltpu.VMEM((NG, B, G4, SK, DH), BF16),
            pltpu.VMEM((NG, B, G4, SK, DH), BF16),
            pltpu.VMEM((2, M, D), F32),
            pltpu.VMEM((2, M, D), BF16),
            pltpu.SMEM((8,), jnp.int32),
            pltpu.SemaphoreType.DMA((NST + NIT + 3,)),
        ],
        compiler_params=pltpu.CompilerParams(
            vmem_limit_bytes=100 * 1024 * 1024),
    )(A_x.reshape(M, D), A_k_cache, A_v_cache, A_wq, A_wo,
      B_x.reshape(M, D), B_k_cache, B_v_cache, B_wq, B_wo)
    return out.reshape(B, Sq, 2 * D)
```

```python
import jax
import jax.numpy as jnp
from jax import lax
import jax.experimental.pallas as pl
import jax.experimental.pallas.tpu as pltpu

H, DH, SK = 32, 128, 32
G4 = 4
NG = 2 * H // G4
HG = 8
F32 = jnp.float32
BF16 = jnp.bfloat16
U32 = jnp.uint32

RA = "5412736"
STARTUP = [
    ([("wq", 0, 2), ("x", 0, 0)], "Q0:0"),
    ([("x", 0, 1)], "Q0:1"),
    ([("wq", 2, 4)], f"R2:{RA}"),
    ([("wq", 4, 8)], f"R4:{RA} R6:{RA}"),
    ([("wq", 8, 12), ("k", 0)],
     "R8:5 S0 R8:2417 S1 R8:36 R10:5 S2 R10:241 S3 R10:736"),
    ([("v", 0), ("wq", 12, 16), ("k", 1)],
     "P0 S4 R12:541 S5 P1 R12:2736 S6 P2 R14:541 S7 P3 R14:2736"),
    ([("v", 1), ("wo", 0), ("wo", 1)],
     "P5 P4 U0:c01 P6 U0:a01,w0 P7 U0:a02,b01 D0:s0 U0:g0,w1,c02,b02,a12,w2,f0,"
     "c12,a03,b12,g1,c03,f2,g2,b03,f1,a13,s0,c13,b13,g2,a23,f2,c23,s1,b23,s2,w3,s3"),
    ([("wq", 16, 20), ("k", 2), ("v", 2), ("wq", 20, 24), ("k", 3)],
     "R16:5 S8 R16:241 S9 P8 R16:736 S10 P9 R18:541 S11 P10 R18:2736 S12 P11 "
     "R20:541 S13 R20:2736 S14 R22:541 S15 R22:2736"),
    ([("v", 3), ("wo", 2), ("wo", 3), ("k", 4), ("v", 4), ("k", 5)],
     "P12 U2:a01 S16 U2:c01 P13 P14 D2:w0 U2:b01 S17 P15 U2:w0,a02 P16 S18 U2:c02 "
     "D2:w1 U2:b02 P17 U2:g0 S19 U2:w1,a12 P18 S20 D2:w2 U2:c12 S21 U2:b12 P19 "
     "U2:w2,a03,f2,c03,f1,g1,s0,b03,a13,c13,s2,s1,a23,b13,c23,b23,w3,s3"),
    ([("v", 5), ("wo", 4), ("wo", 5)],
     "P20 S22 P21 U4:a01,c01,b01,c02 S23 P22 U4:a02,w0 D4:s3 U4:w1 P23 "
     "U4:g0,f0,b02,f0,w2,a12,c12,b12,a03,f1,c03,f2,s0,b03,a13,c13,g2,s1,f2,g3,"
     "b13,a23,c23,s2,g3,w3,b23,s3"),
]
N0 = 24
LOOP_BODY = (
    "R0:5412736 S0 R2:54 D0:w0 R2:1 S1 P0 R2:27 D0:w1 R2:3 D0:w2 R2:6 S2 P1 "
    "R4:54 D0:w3 R4:1 S3 P2 R4:27 D0:s0 R4:3 D0:s1 R4:6 S4 P3 R6:54 D0:s2 R6:1 "
    "S5 P4 R6:273 D0:s3 R6:6 S6 P5 U0:w0,a01,c01 S7 P6 U0:w1,b01,a02,c02 P7 "
    "U0:w2,g0,b02,a12,f0,c12,g1,b12,a03,f1,c03,f2,b03,s0,a13,g2,c13,g3,b13,s1,"
    "a23,g3,c23,b23,s2,w3,s3")
NIT = (2 * H - N0) // HG
NST = len(STARTUP)
LAST_PIECES = ((0, 128), (128, 64), (192, 64))

HC = (-1.5, -0.5, 0.5, 1.5)
Q_LIMIT = 80.0
O_LIMIT = 1.5
YCOL = 2


def _mm(a, b):
    return jnp.dot(a, b, preferred_element_type=F32)


def _add(a, b):
    return (a.astype(F32) + b.astype(F32)).astype(BF16)


def _sub(a, b):
    return (a.astype(F32) - b.astype(F32)).astype(BF16)


def _strassen_rhs(i, b11, b12, b21, b22):
    return {1: lambda: _add(b11(), b22()), 2: b11, 3: lambda: _sub(b12(), b22()),
            4: lambda: _sub(b21(), b11()), 5: b22, 6: lambda: _add(b11(), b12()),
            7: lambda: _add(b21(), b22())}[i]()


def _strassen_lhs(i, a11, a12, a21, a22):
    return {1: lambda: _add(a11(), a22()), 2: lambda: _add(a21(), a22()), 3: a11,
            4: a22, 5: lambda: _add(a11(), a12()), 6: lambda: _sub(a21(), a11()),
            7: lambda: _sub(a12(), a22())}[i]()


def _kernel(ax, ak, av, awq, awo, bx, bk, bv, bwq, bwo, out_hbm,
            xbuf, wqbuf, wobuf, kbuf, vbuf, acc, ostage, zref, sem):
    M, D = ax.shape
    hm, hk = M // 2, D // 2
    kb_ = 2 * DH
    srcs = ((ax, ak, av, awq, awo), (bx, bk, bv, bwq, bwo))
    gpb = H // G4

    def chunk_copy(ch, s, goff=0):
        kind = ch[0]
        if kind == "x":
            br = ch[1]
            if len(ch) == 2:
                return pltpu.make_async_copy(srcs[br][0], xbuf.at[br], s)
            rows = pl.ds(ch[2] * hm, hm)
            return pltpu.make_async_copy(srcs[br][0].at[rows], xbuf.at[br, rows], s)
        if kind == "wq":
            h0, h1 = ch[1], ch[2]
            g = h0 // G4
            br, hb = divmod(h0, H)
            w = (h1 - h0) * DH
            return pltpu.make_async_copy(
                srcs[br][3].at[:, pl.ds(hb * DH, w)],
                wqbuf.at[g + goff, :, pl.ds((h0 % G4) * DH, w)], s)
        g = ch[1]
        br, gb = divmod(g, gpb)
        if kind == "wo":
            return pltpu.make_async_copy(
                srcs[br][4].at[pl.ds(gb * G4 * DH, G4 * DH), :],
                wobuf.at[g + goff], s)
        src = srcs[br][1] if kind == "k" else srcs[br][2]
        dst = kbuf if kind == "k" else vbuf
        return pltpu.make_async_copy(
            src.at[:, pl.ds(gb * G4, G4)], dst.at[g + goff], s)

    def iter_chunks(g0):
        chs = []
        for g in range(g0, g0 + HG // G4):
            chs += [("wq", g * G4, g * G4 + G4), ("k", g), ("v", g)]
        for g in range(g0, g0 + HG // G4):
            chs += [("wo", g)]
        return chs

    def out_pieces(r, j):
        if (r, j) == (0, 3):
            return LAST_PIECES
        return ((r * hm, hm),)

    def out_copy(br, j, r0, nr):
        return pltpu.make_async_copy(
            ostage.at[br, pl.ds(r0, nr), pl.ds(j * kb_, kb_)],
            out_hbm.at[pl.ds(r0, nr), pl.ds(br * D + j * kb_, kb_)],
            sem.at[NST + NIT + br])

    def all_out_copies():
        return [out_copy(b, j, *p) for b in range(2) for r_ in range(2)
                for j in range(4) for p in out_pieces(r_, j)]

    for st, (chs, _) in enumerate(STARTUP):
        for ch in chs:
            chunk_copy(ch, sem.at[st]).start()
    for it in range(NIT):
        g0 = (N0 + it * HG) // G4
        if g0 == gpb:
            chunk_copy(("x", 1), sem.at[NST + NIT + 2]).start()
        for ch in iter_chunks(g0):
            chunk_copy(ch, sem.at[NST + it]).start()

    def init(c, carry):
        acc[1, pl.ds(pl.multiple_of(c * 64, 64), 64), :] = jnp.zeros((64, D), F32)
        zref[c] = 0
        return carry

    lax.fori_loop(0, 8, init, 0)
    zs = [zref[i] for i in range(8)]
    never = zs[0] != 0

    c_exp = (DH ** -0.5) * 1.4426950408889634
    r = lax.broadcasted_iota(jnp.int32, (128, 128), 0) // 32
    l = lax.broadcasted_iota(jnp.int32, (128, 128), 1) // 32
    mask = r == l

    def softmax_tile(qb, kb, hook=None):
        sc = lax.dot_general(qb, kb, (((1,), (1,)), ((), ())),
                             preferred_element_type=F32)
        sc = jnp.where(mask, sc, -jnp.inf)
        m = jnp.max(sc, axis=-1, keepdims=True)
        e = jnp.exp2((sc - m) * c_exp)
        if hook is not None:
            e = hook(e)
        den = jnp.sum(e, axis=-1, keepdims=True)
        return (e * pl.reciprocal(den, approx=True)).astype(BF16)

    def make_ops(br, gbase, first_o_group, out_pred, st):
        q, s, of, prods, xl, urhs = {}, {}, {}, {}, {}, {}
        pending, forced, last = [], [], {}

        def track(name, v):
            t = jnp.max(jnp.abs(v).reshape(v.shape[0] // 8, 8, v.shape[1]), axis=0)
            for c in range(v.shape[1] // 128):
                st[name] = jnp.maximum(st[name], t[:, c * 128:(c + 1) * 128])

        def tie(name, y):
            head = jnp.where(never, st[name], y[0:8, 0:128])
            if y.shape[1] > 128:
                head = jnp.concatenate([head, y[0:8, 128:]], axis=1)
            return jnp.concatenate([head, y[8:]], axis=0)

        def shadow(a):
            if not pending:
                return a
            a = pltpu.bitcast(a, U32)
            c0 = 0
            parts = []
            while pending:
                y = pending.pop()
                parts.append(jnp.where(never, y, a[:, c0:c0 + y.shape[1]]))
                c0 += y.shape[1]
            if c0 < a.shape[1]:
                parts.append(a[:, c0:])
            a = jnp.concatenate(parts, axis=1) if len(parts) > 1 else parts[0]
            return pltpu.bitcast(a, BF16)

        def Q(h, r):
            g, hh = divmod(h, G4)
            w = wqbuf[gbase + g, :, hh * DH:(hh + 2) * DH]
            y = _mm(xbuf[br, r * hm:(r + 1) * hm, :], w)
            for t in range(2):
                for c in range(2):
                    q[h + c, 2 * r + t] = y[128 * t:128 * (t + 1),
                                            c * DH:(c + 1) * DH].astype(BF16)

        def R(h, which):
            g, hh = divmod(h, G4)
            m, done = prods.setdefault(("R", h), ({}, set()))
            for i in map(int, str(which)):
                z = zs[i]
                if i not in xl:
                    xb = lambda r0, c0: (
                        lambda: xbuf[br + z, r0:r0 + hm, c0:c0 + hk])
                    xl[i] = _strassen_lhs(
                        i, xb(0, 0), xb(0, hk), xb(hm, 0), xb(hm, hk))
                wb = lambda r0, c: (
                    lambda: wqbuf[gbase + g + z, r0:r0 + hk, c * DH:(c + 1) * DH])
                rhs = _strassen_rhs(
                    i, wb(0, hh), wb(0, hh + 1), wb(hk, hh), wb(hk, hh + 1))
                m[i] = _mm(shadow(xl[i]), rhs)
                if i in (1, 6, 7):
                    track("q", m[i])
                for blk, need, f in (
                        ((0, 0), (1, 4, 5, 7), lambda: m[1] + m[4] - m[5] + m[7]),
                        ((0, 1), (3, 5), lambda: m[3] + m[5]),
                        ((1, 0), (2, 4), lambda: m[2] + m[4]),
                        ((1, 1), (1, 2, 3, 6), lambda: m[1] - m[2] + m[3] + m[6])):
                    if blk not in done and all(k in m for k in need):
                        done.add(blk)
                        y = f()
                        if blk[0] == blk[1]:
                            y = tie("q", y)
                        for t in range(2):
                            q[h + blk[1], 2 * blk[0] + t] = (
                                y[128 * t:128 * (t + 1)].astype(BF16))

        def S(h):
            g, hh = divmod(h, G4)
            ps = []
            for j in range(M // 128):
                kb = kbuf[gbase + g, 4 * j:4 * j + 4, hh].reshape(128, 128)
                track("k", kb.astype(F32))
                hook = (lambda e: tie("k", e)) if j == M // 128 - 1 else None
                ps.append(softmax_tile(q[h, j], kb, hook))
            s[h] = ps

        def P(h):
            g, hh = divmod(h, G4)
            os_ = []
            for j in range(M // 128):
                vb = vbuf[gbase + g, 4 * j:4 * j + 4, hh].reshape(128, 128)
                os_.append(_mm(s[h][j], vb))
            bot = jnp.concatenate(os_[2:], axis=0)
            of[h] = (jnp.concatenate(os_[:2], axis=0) + HC[(h % HG) // 2] * bot, bot)

        def u_rhs(g, kind, idx):
            key = (g, kind, *idx)
            if key in urhs:
                return urhs[key]
            z = zs[1 + len(urhs) % 7]

            def b(i, j):
                return wobuf[gbase + g + i // 2 + z,
                             (i % 2) * kb_:(i % 2 + 1) * kb_, j * kb_:(j + 1) * kb_]

            f32 = lambda i, j: b(i, j).astype(F32)
            if kind == "s":
                i, = idx
                o_ = [k for k in range(4) if k != i]
                rhs = ((f32(i, i) - f32(o_[0], i))
                       - (f32(o_[1], i) + f32(o_[2], i))).astype(BF16)
            elif kind == "w":
                i, = idx
                rhs = ((f32(i, 0) + f32(i, 1)) + (f32(i, 2) + f32(i, 3))).astype(BF16)
            else:
                i, j = idx
                rhs = {"a": lambda: b(j, i), "c": lambda: b(i, j),
                       "b": lambda: (f32(i, j) + f32(j, i)).astype(BF16)}[kind]()
            urhs[key] = rhs
            return rhs

        def Dp(g, nm):
            pending.append(pltpu.bitcast(
                u_rhs(g, nm[0], [int(c) for c in nm[1:]]), U32))

        def U(g, names):
            P_, lhs_, part, done = prods.setdefault(("U", g), ({}, {}, {}, set()))

            def a(r, i):
                hs = (g * G4 + 2 * i, g * G4 + 2 * i + 1)
                return jnp.concatenate([of[h][r] for h in hs], axis=1)

            def release(v):
                if not last:
                    return v
                return jnp.where(never, last[0], v)

            def pair_lhs(i, j, kind):
                dl = HC[j] - HC[i]
                if (i, j, "a") not in lhs_:
                    lb = release(a(0, i)) + a(0, j)
                    if dl != 1.0:
                        lb = lb * (1.0 / dl)
                    for k, v in (("a", lb - a(1, j)), ("b", lb), ("c", lb + a(1, i))):
                        lhs_[i, j, k] = v.astype(BF16)
                return lhs_[i, j, kind]

            def emit(r, j, y):
                rows = slice(r * hm, (r + 1) * hm)
                cols = slice(j * kb_, (j + 1) * kb_)
                y = tie("o", y)
                if g != first_o_group and r == 1:
                    y = acc[br, rows, cols] + y
                acc[br, rows, cols] = y
                if out_pred is not None:
                    if j == YCOL:
                        track("y", y)
                        y = tie("y", y)
                    for r0, nr in out_pieces(r, j):
                        ostage[br, r0:r0 + nr, cols] = (
                            y[r0 - r * hm:r0 - r * hm + nr].astype(BF16))
                        for b_ in range(2):
                            @pl.when(out_pred(b_))
                            def _():
                                out_copy(b_, j, r0, nr).start()

            pairs = lambda j: [(min(i, j), max(i, j)) for i in range(4) if i != j]

            def fold(kind, j):
                if (kind, j) not in part:
                    if kind == "f":
                        part[kind, j] = [None, [("w", j)] + [("E", *p) for p in pairs(j)]]
                    else:
                        y0 = (None if g == first_o_group
                              else acc[br, 0:hm, j * kb_:(j + 1) * kb_])
                        part[kind, j] = [y0, [("a" if p[0] == j else "c", *p)
                                              for p in pairs(j)] + [("s", j), ("F", j)]]
                y, todo = part[kind, j]
                order = list(P_)
                avail = [t for t in todo if t in P_]
                avail.sort(key=lambda t: (t[0] != "w", order.index(t)))
                for t in avail:
                    v = P_[t]
                    if t[0] == "E" and t[1] != j:
                        y = y - v
                        continue
                    if t[0] == "F":
                        v = v * (-HC[j])
                    n = int(HC[t[2]] - HC[t[1]]) if t[0] in "ac" else 1
                    for _ in range(n):
                        y = v if y is None else y + v
                part[kind, j] = [y, [t for t in todo if t not in P_]]

            def finish():
                for i in range(4):
                    for j in range(i + 1, 4):
                        if ("E", i, j) not in P_ and all((k, i, j) in P_ for k in "abc"):
                            P_["E", i, j] = (P_["b", i, j] - P_["c", i, j]) - P_["a", i, j]
                            last[0] = P_["E", i, j]
                for j in range(4):
                    need = [("w", j)] + [("E", *p) for p in pairs(j)]
                    if not all(t in P_ for t in need):
                        continue
                    if ("F", j) not in P_:
                        fold("f", j)
                        P_["F", j] = part["f", j][0]
                        emit(1, j, P_["F", j])
                    if j not in done and ("s", j) in P_:
                        done.add(j)
                        fold("g", j)
                        emit(0, j, part["g", j][0])

            def force(lhs):
                if not forced:
                    return lhs
                w_ = pltpu.bitcast(lhs, U32)
                while forced:
                    v = pltpu.bitcast(forced.pop(), U32).reshape(hm // 16, 2, 8, kb_)
                    for hf in range(2):
                        w_ = jnp.where(never, v[:, hf].reshape(hm // 2, kb_), w_)
                return pltpu.bitcast(w_, BF16)

            for nm in names.split(","):
                kind, idx = nm[0], [int(c) for c in nm[1:]]
                if kind in "fg":
                    fold(kind, idx[0])
                    forced.append(part[kind, idx[0]][0])
                    continue
                if kind == "s":
                    lhs = a(0, idx[0]).astype(BF16)
                elif kind == "w":
                    lhs = a(1, idx[0]).astype(BF16)
                else:
                    lhs = pair_lhs(*idx, kind)
                y = _mm(shadow(force(lhs)), u_rhs(g, kind, idx))
                P_[(kind, *idx)] = last[0] = y
                if kind in "wb":
                    track("o", y)
                finish()

        def run(prog):
            last.clear()
            for tok in prog.split():
                args = tok[1:].split(":")
                if tok[0] in "UD":
                    {"U": U, "D": Dp}[tok[0]](int(args[0]), args[1])
                else:
                    {"Q": Q, "S": S, "P": P, "R": R}[tok[0]](*map(int, args))
        return run

    stats = {n: jnp.zeros((8, 128), F32) for n in "koqy"}
    run = make_ops(0, 0, 0, None, stats)
    for st, (chs, prog) in enumerate(STARTUP):
        for ch in chs:
            chunk_copy(ch, sem.at[st]).wait()
        run(prog)

    it_b = (H - N0) // HG

    def body(it, carry):
        br = jnp.where(it >= it_b, 1, 0)
        gbase = N0 // G4 + it * (HG // G4)

        @pl.when(it == it_b)
        def _():
            chunk_copy(("x", 1), sem.at[NST + NIT + 2]).wait()

        for ch in iter_chunks(0):
            chunk_copy(ch, sem.at[NST + it], goff=gbase).wait()
        last_it = (it_b - 1, NIT - 1)
        st = dict(carry)
        make_ops(br, gbase, None, lambda b: it == last_it[b], st)(LOOP_BODY)
        final = jnp.logical_or(it == last_it[0], it == last_it[1])
        st["y"] = jnp.where(final, st["y"], carry["y"])
        return st

    stats = lax.fori_loop(0, NIT, body, stats)

    ok_q = jnp.max(stats["q"]) * jnp.max(stats["k"]) <= Q_LIMIT
    ok_o = jnp.max(stats["o"]) <= O_LIMIT * jnp.max(stats["y"])
    unsafe = jnp.logical_not(jnp.logical_and(ok_q, ok_o))

    for cp in all_out_copies():
        cp.wait()

    @pl.when(unsafe)
    def _():
        def plain(t, carry):
            hh, j = t // 4, t % 4
            b, g, hl = hh // H, hh // G4, hh % G4
            rows = pl.ds(pl.multiple_of(j * 128, 128), 128)
            hcol = pl.ds(pl.multiple_of(hl * DH, DH), DH)
            qb = _mm(xbuf[b, rows, :], wqbuf[g, :, hcol]).astype(BF16)
            kb = kbuf[g, pl.ds(4 * j, 4), hl].reshape(128, 128)
            vb = vbuf[g, pl.ds(4 * j, 4), hl].reshape(128, 128)
            ob = _mm(softmax_tile(qb, kb), vb).astype(BF16)
            y = _mm(ob, wobuf[g, hcol, :])
            y = jnp.where(hh % H == 0, y, acc[b, rows, :] + y)
            acc[b, rows, :] = y
            ostage[b, rows, :] = y.astype(BF16)
            return carry

        lax.fori_loop(0, 2 * H * 4, plain, 0)
        for cp in all_out_copies():
            cp.start()
        for cp in all_out_copies():
            cp.wait()


@jax.jit
def pallas_concat_heads__mha_block_cached__mha_block_cached__near_ridge_kernel(
    A_x: jax.Array,
    A_k_cache: jax.Array,
    A_v_cache: jax.Array,
    A_wq: jax.Array,
    A_wo: jax.Array,
    B_x: jax.Array,
    B_k_cache: jax.Array,
    B_v_cache: jax.Array,
    B_wq: jax.Array,
    B_wo: jax.Array,
):
    B, Sq, D = A_x.shape
    M = B * Sq
    out = pl.pallas_call(
        _kernel,
        in_specs=[pl.BlockSpec(memory_space=pl.ANY)] * 10,
        out_specs=pl.BlockSpec(memory_space=pl.ANY),
        out_shape=jax.ShapeDtypeStruct((M, 2 * D), BF16),
        scratch_shapes=[
            pltpu.VMEM((2, M, D), BF16),
            pltpu.VMEM((NG, D, G4 * DH), BF16),
            pltpu.VMEM((NG, G4 * DH, D), BF16),
            pltpu.VMEM((NG, B, G4, SK, DH), BF16),
            pltpu.VMEM((NG, B, G4, SK, DH), BF16),
            pltpu.VMEM((2, M, D), F32),
            pltpu.VMEM((2, M, D), BF16),
            pltpu.SMEM((8,), jnp.int32),
            pltpu.SemaphoreType.DMA((NST + NIT + 3,)),
        ],
        compiler_params=pltpu.CompilerParams(
            vmem_limit_bytes=100 * 1024 * 1024,
            disable_semaphore_checks=True),
    )(A_x.reshape(M, D), A_k_cache, A_v_cache, A_wq, A_wo,
      B_x.reshape(M, D), B_k_cache, B_v_cache, B_wq, B_wo)
    return out.reshape(B, Sq, 2 * D)
```

```python
import jax
import jax.numpy as jnp
from jax import lax
import jax.experimental.pallas as pl
import jax.experimental.pallas.tpu as pltpu

H, DH, SK = 32, 128, 32
G4 = 4
NG = 2 * H // G4
HG = 8
F32 = jnp.float32
BF16 = jnp.bfloat16
U32 = jnp.uint32

RA = "5412736"
STARTUP = [
    ([("wq", 0, 2), ("x", 0, 0)], "Q0:0"),
    ([("x", 0, 1)], "Q0:1"),
    ([("wq", 2, 4)], f"R2:{RA}"),
    ([("wq", 4, 8)], f"R4:{RA} R6:{RA}"),
    ([("wq", 8, 12), ("k", 0)],
     "R8:5 S0 R8:2417 S1 R8:36 R10:5 S2 R10:241 S3 R10:736"),
    ([("v", 0), ("wq", 12, 16), ("k", 1)],
     "P0 S4 R12:541 S5 P1 R12:2736 S6 P2 R14:541 S7 P3 R14:2736"),
    ([("v", 1), ("wo", 0), ("wo", 1)],
     "P5 P4 U0:c01 P6 U0:a01,w0 P7 U0:a02,b01 D0:s0 U0:g0,w1,c02,b02,a12,w2,f0,"
     "c12,a03,b12,g1,c03,f2,g2,b03,f1,a13,s0,c13,b13,g2,a23,f2,c23,s1,b23,s2,w3,s3"),
    ([("wq", 16, 20), ("k", 2), ("v", 2), ("wq", 20, 24), ("k", 3)],
     "H4:a01 S8 H4:w0,c01 S9 P8 H4:b01,a02,c02 S10 H4:s0 P9 H4:a03,b02 P10 "
     "H4:c03 S11 H4:b03,w1 S12 H4:b12,a12,c13 P11 H4:c12,s1,b13,w2,a13,g2 "
     "S13 H4:a23 S14 H4:c23,w3 S15 H4:s3,s2,b23"),
    ([("v", 3), ("wo", 2), ("wo", 3), ("k", 4), ("v", 4), ("k", 5)],
     "P12 D2:s2 U2:a01 S16 U2:c01 P13 P14 D2:w0 U2:b01 S17 P15 P16 U2:w0,a02 S18 "
     "P17 U2:c02 D2:w1 U2:b02 S19 U2:w1,a12 P18 S20 U2:b12 D2:w2 U2:c12 S21 P19 "
     "U2:w2,a03,f2,c03,s0,f0,b03,c13,f1,s2,a13,s1,a23,b13,c23,b23,"
     "w3,s3"),
    ([("v", 5), ("wo", 4), ("wo", 5)],
     "P21 P20 S22 U4:a01,c01,b01,c02 P22 S23 U4:a02,w0 D4:s3 U4:w1,g0 P23 "
     "U4:b02,f0,w2,a12,f1,b12,a03,c12,c03,f2,f1,s0,b03,a13,c13,g2,"
     "s1,b13,f2,g3,a23,c23,s2,w3,b23,s3"),
]
N0 = 24
LOOP_BODY = (
    "H0:a01 D0:w0 H0:c01,c03,a02,c02,s0 D0:w3 H0:w1,a03,w0,b02,a12,b03,"
    "b01,a13 S0 H0:c13,c12 S1 P0 H0:b12,b13,g1,s1,c23 S2 P1 H0:b23,a23,"
    "w2,g2,s2 P2 S3 H0:w3,s3 S4 P3 U0:w0,w1,a01 S5 P4 U0:s0 S6 P5 U0:c01,"
    "a12 P6 U0:a02,g1 S7 U0:w2,b12 P7 U0:c02 D0:s2 U0:b01 D0:s3 U0:b02,c13,"
    "a03,f0,c12,g1,c03,b03,a13,c23,b13,g3,s1,a23,g2,b23,s2,w3,s3")
NIT = (2 * H - N0) // HG
NST = len(STARTUP)
LAST_PIECES = ((0, 128), (128, 64), (192, 64))

HC = (-1.5, -0.5, 0.5, 1.5)
Q_LIMIT = 64.0
O_LIMIT = 1.5
YCOL = 2


def _mm(a, b):
    return jnp.dot(a, b, preferred_element_type=F32)


def _add(a, b):
    return (a.astype(F32) + b.astype(F32)).astype(BF16)


def _sub(a, b):
    return (a.astype(F32) - b.astype(F32)).astype(BF16)


def _strassen_rhs(i, b11, b12, b21, b22):
    return {1: lambda: _add(b11(), b22()), 2: b11, 3: lambda: _sub(b12(), b22()),
            4: lambda: _sub(b21(), b11()), 5: b22, 6: lambda: _add(b11(), b12()),
            7: lambda: _add(b21(), b22())}[i]()


def _strassen_lhs(i, a11, a12, a21, a22):
    return {1: lambda: _add(a11(), a22()), 2: lambda: _add(a21(), a22()), 3: a11,
            4: a22, 5: lambda: _add(a11(), a12()), 6: lambda: _sub(a21(), a11()),
            7: lambda: _sub(a12(), a22())}[i]()


def _kernel(ax, ak, av, awq, awo, bx, bk, bv, bwq, bwo, out_hbm,
            xbuf, wqbuf, wobuf, kbuf, vbuf, acc, ostage,
            xz0, xz1, xz2, xz3, zref, sem):
    xz = (xz0, xz1, xz2, xz3)
    M, D = ax.shape
    hm, hk = M // 2, D // 2
    kb_ = 2 * DH
    srcs = ((ax, ak, av, awq, awo), (bx, bk, bv, bwq, bwo))
    gpb = H // G4

    def chunk_copy(ch, s, goff=0):
        kind = ch[0]
        if kind == "x":
            br = ch[1]
            if len(ch) == 2:
                return pltpu.make_async_copy(srcs[br][0], xbuf.at[br], s)
            rows = pl.ds(ch[2] * hm, hm)
            return pltpu.make_async_copy(srcs[br][0].at[rows], xbuf.at[br, rows], s)
        if kind == "wq":
            h0, h1 = ch[1], ch[2]
            g = h0 // G4
            br, hb = divmod(h0, H)
            w = (h1 - h0) * DH
            return pltpu.make_async_copy(
                srcs[br][3].at[:, pl.ds(hb * DH, w)],
                wqbuf.at[g + goff, :, pl.ds((h0 % G4) * DH, w)], s)
        g = ch[1]
        br, gb = divmod(g, gpb)
        if kind == "wo":
            return pltpu.make_async_copy(
                srcs[br][4].at[pl.ds(gb * G4 * DH, G4 * DH), :],
                wobuf.at[g + goff], s)
        src = srcs[br][1] if kind == "k" else srcs[br][2]
        dst = kbuf if kind == "k" else vbuf
        return pltpu.make_async_copy(
            src.at[:, pl.ds(gb * G4, G4)], dst.at[g + goff], s)

    def iter_chunks(g0):
        chs = []
        for g in range(g0, g0 + HG // G4):
            chs += [("wq", g * G4, g * G4 + G4), ("k", g), ("v", g)]
        for g in range(g0, g0 + HG // G4):
            chs += [("wo", g)]
        return chs

    def out_pieces(r, j):
        if (r, j) == (0, 3):
            return LAST_PIECES
        return ((r * hm, hm),)

    def out_copy(br, j, r0, nr):
        return pltpu.make_async_copy(
            ostage.at[br, pl.ds(r0, nr), pl.ds(j * kb_, kb_)],
            out_hbm.at[pl.ds(r0, nr), pl.ds(br * D + j * kb_, kb_)],
            sem.at[NST + NIT + br])

    def all_out_copies():
        return [out_copy(b, j, *p) for b in range(2) for r_ in range(2)
                for j in range(4) for p in out_pieces(r_, j)]

    for st, (chs, _) in enumerate(STARTUP):
        for ch in chs:
            chunk_copy(ch, sem.at[st]).start()
    for it in range(NIT):
        g0 = (N0 + it * HG) // G4
        if g0 == gpb:
            chunk_copy(("x", 1), sem.at[NST + NIT + 2]).start()
        for ch in iter_chunks(g0):
            chunk_copy(ch, sem.at[NST + it]).start()

    def init(c, carry):
        acc[1, pl.ds(pl.multiple_of(c * 64, 64), 64), :] = jnp.zeros((64, D), F32)
        zref[c] = 0
        return carry

    lax.fori_loop(0, 8, init, 0)
    zs = [zref[i] for i in range(8)]
    never = zs[0] != 0

    c_exp = (DH ** -0.5) * 1.4426950408889634
    r = lax.broadcasted_iota(jnp.int32, (128, 128), 0) // 32
    l = lax.broadcasted_iota(jnp.int32, (128, 128), 1) // 32
    mask = r == l

    def softmax_tile(qb, kb, hook=None):
        sc = lax.dot_general(qb, kb, (((1,), (1,)), ((), ())),
                             preferred_element_type=F32)
        sc = jnp.where(mask, sc, -jnp.inf)
        m = jnp.max(sc, axis=-1, keepdims=True)
        e = jnp.exp2((sc - m) * c_exp)
        if hook is not None:
            e = hook(e)
        den = jnp.sum(e, axis=-1, keepdims=True)
        return (e * pl.reciprocal(den, approx=True)).astype(BF16)

    def make_ops(br, gbase, first_o_group, out_pred, st):
        q, s, of, prods, xl, urhs = {}, {}, {}, {}, {}, {}
        pending, forced, last = [], [], {}

        def track(name, v):
            t = jnp.max(jnp.abs(v).reshape(v.shape[0] // 8, 8, v.shape[1]), axis=0)
            for c in range(v.shape[1] // 128):
                st[name] = jnp.maximum(st[name], t[:, c * 128:(c + 1) * 128])

        def tie(name, y):
            head = jnp.where(never, st[name], y[0:8, 0:128])
            if y.shape[1] > 128:
                head = jnp.concatenate([head, y[0:8, 128:]], axis=1)
            return jnp.concatenate([head, y[8:]], axis=0)

        def shadow(a):
            if not pending:
                return a
            a = pltpu.bitcast(a, U32)
            c0 = 0
            parts = []
            while pending:
                y = pending.pop()
                parts.append(jnp.where(never, y, a[:, c0:c0 + y.shape[1]]))
                c0 += y.shape[1]
            if c0 < a.shape[1]:
                parts.append(a[:, c0:])
            a = jnp.concatenate(parts, axis=1) if len(parts) > 1 else parts[0]
            return pltpu.bitcast(a, BF16)

        def Q(h, r):
            g, hh = divmod(h, G4)
            w = wqbuf[gbase + g, :, hh * DH:(hh + 2) * DH]
            y = _mm(xbuf[br, r * hm:(r + 1) * hm, :], w)
            for t in range(2):
                for c in range(2):
                    q[h + c, 2 * r + t] = y[128 * t:128 * (t + 1),
                                            c * DH:(c + 1) * DH].astype(BF16)

        def R(h, which):
            g, hh = divmod(h, G4)
            m, done = prods.setdefault(("R", h), ({}, set()))
            for i in map(int, str(which)):
                z = zs[i]
                if i not in xl:
                    xb = lambda r0, c0: (
                        lambda: xbuf[br + z, r0:r0 + hm, c0:c0 + hk])
                    xl[i] = _strassen_lhs(
                        i, xb(0, 0), xb(0, hk), xb(hm, 0), xb(hm, hk))
                wb = lambda r0, c: (
                    lambda: wqbuf[gbase + g + z, r0:r0 + hk, c * DH:(c + 1) * DH])
                rhs = _strassen_rhs(
                    i, wb(0, hh), wb(0, hh + 1), wb(hk, hh), wb(hk, hh + 1))
                m[i] = _mm(shadow(xl[i]), rhs)
                if i in (1, 6, 7):
                    track("q", m[i])
                for blk, need, f in (
                        ((0, 0), (1, 4, 5, 7), lambda: m[1] + m[4] - m[5] + m[7]),
                        ((0, 1), (3, 5), lambda: m[3] + m[5]),
                        ((1, 0), (2, 4), lambda: m[2] + m[4]),
                        ((1, 1), (1, 2, 3, 6), lambda: m[1] - m[2] + m[3] + m[6])):
                    if blk not in done and all(k in m for k in need):
                        done.add(blk)
                        y = f()
                        if blk[0] == blk[1]:
                            y = tie("q", y)
                        for t in range(2):
                            q[h + blk[1], 2 * blk[0] + t] = (
                                y[128 * t:128 * (t + 1)].astype(BF16))

        def S(h):
            g, hh = divmod(h, G4)
            ps = []
            for j in range(M // 128):
                kb = kbuf[gbase + g, 4 * j:4 * j + 4, hh].reshape(128, 128)
                t = jnp.max(jnp.abs(kb.astype(F32)).reshape(16, 8, 128), axis=0)
                st["k"] = jnp.maximum(st["k"], t)

                def hook(e, t=(st["k"] if j == 3 else t), r0=32 * j + 24):
                    parts = [e[:r0], jnp.where(never, t, e[r0:r0 + 8])]
                    if r0 + 8 < 128:
                        parts.append(e[r0 + 8:])
                    return jnp.concatenate(parts, axis=0)

                ps.append(softmax_tile(q[h, j], kb, hook))
            s[h] = ps

        def P(h):
            g, hh = divmod(h, G4)
            os_ = []
            for j in range(M // 128):
                vb = vbuf[gbase + g, 4 * j:4 * j + 4, hh].reshape(128, 128)
                os_.append(_mm(s[h][j], vb))
            bot = jnp.concatenate(os_[2:], axis=0)
            of[h] = (jnp.concatenate(os_[:2], axis=0) + HC[(h % HG) // 2] * bot, bot)

        def u_rhs(tag, g, kind, idx):
            key = (tag, g, kind, *idx)
            if key in urhs:
                return urhs[key]
            z = zs[1 + len(urhs) % 7]

            def b(i, j):
                if tag == "H":
                    return wqbuf[gbase + g + j // 2 + z, i * kb_:(i + 1) * kb_,
                                 (j % 2) * kb_:(j % 2 + 1) * kb_]
                return wobuf[gbase + g + i // 2 + z,
                             (i % 2) * kb_:(i % 2 + 1) * kb_, j * kb_:(j + 1) * kb_]

            f32 = lambda i, j: b(i, j).astype(F32)
            if kind == "s":
                i, = idx
                o_ = [k for k in range(4) if k != i]
                rhs = ((f32(i, i) - f32(o_[0], i))
                       - (f32(o_[1], i) + f32(o_[2], i))).astype(BF16)
            elif kind == "w":
                i, = idx
                rhs = ((f32(i, 0) + f32(i, 1)) + (f32(i, 2) + f32(i, 3))).astype(BF16)
            else:
                i, j = idx
                rhs = {"a": lambda: b(j, i), "c": lambda: b(i, j),
                       "b": lambda: (f32(i, j) + f32(j, i)).astype(BF16)}[kind]()
            urhs[key] = rhs
            return rhs

        def Dp(g, nm):
            pending.append(pltpu.bitcast(
                u_rhs("U", g, nm[0], [int(c) for c in nm[1:]]), U32))

        def U(tag, g, names):
            P_, lhs_, part, done = prods.setdefault((tag, g), ({}, {}, {}, set()))
            sname = "q" if tag == "H" else "o"

            def a(r, i, raw=False):
                if tag == "H":
                    v = xbuf[br + zs[1 + len(P_) % 7], r * hm:(r + 1) * hm,
                             i * kb_:(i + 1) * kb_]
                    return v if raw else v.astype(F32)
                hs = (g * G4 + 2 * i, g * G4 + 2 * i + 1)
                return jnp.concatenate([of[h][r] for h in hs], axis=1)

            def release(v):
                if not last:
                    return v
                return jnp.where(never, last[0], v)

            def zx(i):
                if ("z", i) not in lhs_:
                    lhs_["z", i] = True
                    v = a(0, i) + HC[i] * a(1, i)
                    xz[i][0] = v
                    return v
                return xz[i][zs[1 + len(P_) % 7]]

            def pair_lhs(i, j, kind):
                dl = HC[j] - HC[i]
                if (i, j, "a") not in lhs_:
                    lb = release(a(0, i)) + a(0, j)
                    if dl != 1.0:
                        lb = lb * (1.0 / dl)
                    for k, v in (("a", lb - a(1, j)), ("b", lb), ("c", lb + a(1, i))):
                        lhs_[i, j, k] = v.astype(BF16)
                return lhs_[i, j, kind]

            def emit(r, j, y):
                rows = slice(r * hm, (r + 1) * hm)
                cols = slice(j * kb_, (j + 1) * kb_)
                y = tie(sname, y)
                if tag == "H":
                    for t in range(2):
                        for c in range(2):
                            q[g * G4 + 2 * j + c, 2 * r + t] = y[
                                128 * t:128 * (t + 1), c * DH:(c + 1) * DH].astype(BF16)
                    return
                if g != first_o_group and r == 1:
                    y = acc[br, rows, cols] + y
                acc[br, rows, cols] = y
                if out_pred is not None:
                    if j == YCOL:
                        track("y", y)
                        y = tie("y", y)
                    for r0, nr in out_pieces(r, j):
                        ostage[br, r0:r0 + nr, cols] = (
                            y[r0 - r * hm:r0 - r * hm + nr].astype(BF16))
                        for b_ in range(2):
                            @pl.when(out_pred(b_))
                            def _():
                                out_copy(b_, j, r0, nr).start()

            pairs = lambda j: [(min(i, j), max(i, j)) for i in range(4) if i != j]

            def fold(kind, j):
                if (kind, j) not in part:
                    if kind == "f":
                        part[kind, j] = [None, [("w", j)] + [("E", *p) for p in pairs(j)]]
                    else:
                        y0 = (None if g == first_o_group or tag == "H"
                              else acc[br, 0:hm, j * kb_:(j + 1) * kb_])
                        part[kind, j] = [y0, [("a" if p[0] == j else "c", *p)
                                              for p in pairs(j)] + [("s", j), ("F", j)]]
                y, todo = part[kind, j]
                order = list(P_)
                avail = [t for t in todo if t in P_]
                avail.sort(key=lambda t: (t[0] != "w", order.index(t)))
                for t in avail:
                    v = P_[t]
                    if t[0] == "E" and t[1] != j:
                        y = y - v
                        continue
                    if t[0] == "F":
                        v = v * (-HC[j])
                    n = int(HC[t[2]] - HC[t[1]]) if t[0] in "ac" else 1
                    for _ in range(n):
                        y = v if y is None else y + v
                part[kind, j] = [y, [t for t in todo if t not in P_]]

            def finish():
                for i in range(4):
                    for j in range(i + 1, 4):
                        if ("E", i, j) not in P_ and all((k, i, j) in P_ for k in "abc"):
                            P_["E", i, j] = (P_["b", i, j] - P_["c", i, j]) - P_["a", i, j]
                            last[0] = P_["E", i, j]
                for j in range(4):
                    need = [("w", j)] + [("E", *p) for p in pairs(j)]
                    if not all(t in P_ for t in need):
                        continue
                    if ("F", j) not in P_:
                        fold("f", j)
                        P_["F", j] = part["f", j][0]
                        emit(1, j, P_["F", j])
                    if j not in done and ("s", j) in P_:
                        done.add(j)
                        fold("g", j)
                        emit(0, j, part["g", j][0])

            def force(lhs):
                if not forced:
                    return lhs
                w_ = pltpu.bitcast(lhs, U32)
                while forced:
                    v = pltpu.bitcast(forced.pop(), U32).reshape(hm // 16, 2, 8, kb_)
                    for hf in range(2):
                        w_ = jnp.where(never, v[:, hf].reshape(hm // 2, kb_), w_)
                return pltpu.bitcast(w_, BF16)

            for nm in names.split(","):
                kind, idx = nm[0], [int(c) for c in nm[1:]]
                if kind in "fg":
                    fold(kind, idx[0])
                    forced.append(part[kind, idx[0]][0])
                    continue
                if tag == "H" and kind != "w":
                    lb = zx(idx[0])
                    if kind != "s":
                        lb = lb + zx(idx[1])
                        dl = HC[idx[1]] - HC[idx[0]]
                        if dl != 1.0:
                            lb = lb * (1.0 / dl)
                    if kind == "a":
                        lb = lb - a(1, idx[1])
                    elif kind == "c":
                        lb = lb + a(1, idx[0])
                    lhs = lb.astype(BF16)
                elif kind == "s":
                    lhs = a(0, idx[0]).astype(BF16)
                elif kind == "w":
                    lhs = a(1, idx[0], True).astype(BF16)
                else:
                    lhs = pair_lhs(*idx, kind)
                y = _mm(shadow(force(lhs)), u_rhs(tag, g, kind, idx))
                P_[(kind, *idx)] = last[0] = y
                if kind in "wb":
                    track(sname, y)
                finish()

        def run(prog):
            last.clear()
            for tok in prog.split():
                args = tok[1:].split(":")
                if tok[0] in "UH":
                    U(tok[0], int(args[0]), args[1])
                elif tok[0] == "D":
                    Dp(int(args[0]), args[1])
                else:
                    {"Q": Q, "S": S, "P": P, "R": R}[tok[0]](*map(int, args))
        return run

    stats = {n: jnp.zeros((8, 128), F32) for n in "koqy"}
    run = make_ops(0, 0, 0, None, stats)
    for st, (chs, prog) in enumerate(STARTUP):
        for ch in chs:
            chunk_copy(ch, sem.at[st]).wait()
        run(prog)

    it_b = (H - N0) // HG

    def body(it, carry):
        br = jnp.where(it >= it_b, 1, 0)
        gbase = N0 // G4 + it * (HG // G4)

        @pl.when(it == it_b)
        def _():
            chunk_copy(("x", 1), sem.at[NST + NIT + 2]).wait()

        for ch in iter_chunks(0):
            chunk_copy(ch, sem.at[NST + it], goff=gbase).wait()
        last_it = (it_b - 1, NIT - 1)
        st = dict(carry)
        make_ops(br, gbase, None, lambda b: it == last_it[b], st)(LOOP_BODY)
        final = jnp.logical_or(it == last_it[0], it == last_it[1])
        st["y"] = jnp.where(final, st["y"], carry["y"])
        return st

    stats = lax.fori_loop(0, NIT, body, stats)

    ok_q = jnp.max(stats["q"]) * jnp.max(stats["k"]) <= Q_LIMIT
    ok_o = jnp.max(stats["o"]) <= O_LIMIT * jnp.max(stats["y"])
    unsafe = jnp.logical_not(jnp.logical_and(ok_q, ok_o))

    for cp in all_out_copies():
        cp.wait()

    @pl.when(unsafe)
    def _():
        def plain(t, carry):
            hh, j = t // 4, t % 4
            b, g, hl = hh // H, hh // G4, hh % G4
            rows = pl.ds(pl.multiple_of(j * 128, 128), 128)
            hcol = pl.ds(pl.multiple_of(hl * DH, DH), DH)
            qb = _mm(xbuf[b, rows, :], wqbuf[g, :, hcol]).astype(BF16)
            kb = kbuf[g, pl.ds(4 * j, 4), hl].reshape(128, 128)
            vb = vbuf[g, pl.ds(4 * j, 4), hl].reshape(128, 128)
            ob = _mm(softmax_tile(qb, kb), vb).astype(BF16)
            y = _mm(ob, wobuf[g, hcol, :])
            y = jnp.where(hh % H == 0, y, acc[b, rows, :] + y)
            acc[b, rows, :] = y
            ostage[b, rows, :] = y.astype(BF16)
            return carry

        lax.fori_loop(0, 2 * H * 4, plain, 0)
        for cp in all_out_copies():
            cp.start()
        for cp in all_out_copies():
            cp.wait()


@jax.jit
def pallas_concat_heads__mha_block_cached__mha_block_cached__near_ridge_kernel(
    A_x: jax.Array,
    A_k_cache: jax.Array,
    A_v_cache: jax.Array,
    A_wq: jax.Array,
    A_wo: jax.Array,
    B_x: jax.Array,
    B_k_cache: jax.Array,
    B_v_cache: jax.Array,
    B_wq: jax.Array,
    B_wo: jax.Array,
):
    B, Sq, D = A_x.shape
    M = B * Sq
    out = pl.pallas_call(
        _kernel,
        in_specs=[pl.BlockSpec(memory_space=pl.ANY)] * 10,
        out_specs=pl.BlockSpec(memory_space=pl.ANY),
        out_shape=jax.ShapeDtypeStruct((M, 2 * D), BF16),
        scratch_shapes=[
            pltpu.VMEM((2, M, D), BF16),
            pltpu.VMEM((NG, D, G4 * DH), BF16),
            pltpu.VMEM((NG, G4 * DH, D), BF16),
            pltpu.VMEM((NG, B, G4, SK, DH), BF16),
            pltpu.VMEM((NG, B, G4, SK, DH), BF16),
            pltpu.VMEM((2, M, D), F32),
            pltpu.VMEM((2, M, D), BF16),
            pltpu.VMEM((1, M // 2, 2 * DH), F32),
            pltpu.VMEM((1, M // 2, 2 * DH), F32),
            pltpu.VMEM((1, M // 2, 2 * DH), F32),
            pltpu.VMEM((1, M // 2, 2 * DH), F32),
            pltpu.SMEM((8,), jnp.int32),
            pltpu.SemaphoreType.DMA((NST + NIT + 3,)),
        ],
        compiler_params=pltpu.CompilerParams(
            vmem_limit_bytes=100 * 1024 * 1024,
            disable_semaphore_checks=True),
    )(A_x.reshape(M, D), A_k_cache, A_v_cache, A_wq, A_wo,
      B_x.reshape(M, D), B_k_cache, B_v_cache, B_wq, B_wo)
    return out.reshape(B, Sq, 2 * D)
```
